```python
import os as _os
_os.environ.setdefault("JAX_PLATFORMS", "cpu")
import jax
import jax.numpy as jnp

def _softmax(x, axis=-1):
    return jax.nn.softmax(x, axis=axis)
def _gelu(x):
    return jax.nn.gelu(x, approximate=True)
def _silu(x):
    return jax.nn.silu(x)
def _sigmoid(x):
    return jax.nn.sigmoid(x)
def _layernorm(x, axis=-1, eps=1e-5):
    m = jnp.mean(x, axis=axis, keepdims=True)
    v = jnp.var(x, axis=axis, keepdims=True)
    return (x - m) / jnp.sqrt(v + eps)
def _scatter_add(tgt, idx, src, axis=0):
    return tgt.at[idx].add(src)
def _segment_sum(src, seg, n):
    return jax.ops.segment_sum(src, seg, n)
class _Rng:
    def __init__(self, key):
        self._k = key
    def _next(self):
        self._k, sub = jax.random.split(self._k)
        return sub
    def normal(self, shape):
        return jax.random.normal(self._next(), shape, dtype=jnp.bfloat16)
    def randint(self, lo, hi, shape):
        return jax.random.randint(self._next(), shape, lo, hi, dtype=jnp.int32)
    def uniform(self, shape, lo=0.0, hi=1.0):
        return jax.random.uniform(self._next(), shape, jnp.bfloat16, lo, hi)
    def permutation(self, n):
        return jax.random.permutation(self._next(), n)


kernel_name = 'concat_heads__mha_block_cached__mha_block_cached__near_ridge'

def setup_inputs():
    _rng = _Rng(jax.random.key(int.from_bytes(__import__("os").urandom(4), "little")))
    _w = (lambda a: (lambda t: t.astype(jnp.bfloat16) if jnp.issubdtype(t.dtype, jnp.floating) else t)(jnp.asarray(a)))
    def _A_setup():
        B, Sq, D = 16, 80, 512
        H, Sk, Dh = 32, 80, 128
        return {
            "x": _w((lambda *s: _rng.normal(s) * 0.8)(B, Sq, D)),
            "k_cache": _w((lambda *s: _rng.normal(s) * 0.8)(B, H, Sk, Dh)),
            "v_cache": _w((lambda *s: _rng.normal(s) * 0.05)(B, H, Sk, Dh)),
            "wq": _w((lambda *s: _rng.normal(s) * 0.8)(D, H * Dh) * (D ** -0.5)),
            "wo": _w((lambda *s: _rng.normal(s) * 0.05)(H * Dh, D) * ((H * Dh) ** -0.5)),
        }
    _A_in = _A_setup()

    def _B_setup():
        B, Sq, D = 16, 80, 512
        H, Sk, Dh = 32, 80, 128
        return {
            "x": _w((lambda *s: _rng.normal(s) * 0.8)(B, Sq, D)),
            "k_cache": _w((lambda *s: _rng.normal(s) * 0.8)(B, H, Sk, Dh)),
            "v_cache": _w((lambda *s: _rng.normal(s) * 0.05)(B, H, Sk, Dh)),
            "wq": _w((lambda *s: _rng.normal(s) * 0.8)(D, H * Dh) * (D ** -0.5)),
            "wo": _w((lambda *s: _rng.normal(s) * 0.05)(H * Dh, D) * ((H * Dh) ** -0.5)),
        }
    _B_in = _B_setup()

    return {
        "A_x": _A_in["x"],
        "A_k_cache": _A_in["k_cache"],
        "A_v_cache": _A_in["v_cache"],
        "A_wq": _A_in["wq"],
        "A_wo": _A_in["wo"],
        "B_x": _B_in["x"],
        "B_k_cache": _B_in["k_cache"],
        "B_v_cache": _B_in["v_cache"],
        "B_wq": _B_in["wq"],
        "B_wo": _B_in["wo"],
    }

def reference(A_x, A_k_cache, A_v_cache, A_wq, A_wo, B_x, B_k_cache, B_v_cache, B_wq, B_wo):
    def _A_ref(x, k_cache, v_cache, wq, wo):
        B, Sq, D = x.shape
        H, Dh = 32, 128
        q = (lambda x, *d: x.transpose(*d))((x @ wq).reshape(B, Sq, H, Dh), 0, 2, 1, 3)
        scores = jnp.einsum("bhqd,bhkd->bhqk", q, k_cache) * (Dh ** -0.5)
        p = _softmax(scores, axis=-1)
        o = jnp.einsum("bhqk,bhkd->bhqd", p, v_cache)
        return (lambda x, *d: x.transpose(*d))(o, 0, 2, 1, 3).reshape(B, Sq, H * Dh) @ wo

    def _B_ref(x, k_cache, v_cache, wq, wo):
        B, Sq, D = x.shape
        H, Dh = 32, 128
        q = (lambda x, *d: x.transpose(*d))((x @ wq).reshape(B, Sq, H, Dh), 0, 2, 1, 3)
        scores = jnp.einsum("bhqd,bhkd->bhqk", q, k_cache) * (Dh ** -0.5)
        p = _softmax(scores, axis=-1)
        o = jnp.einsum("bhqk,bhkd->bhqd", p, v_cache)
        return (lambda x, *d: x.transpose(*d))(o, 0, 2, 1, 3).reshape(B, Sq, H * Dh) @ wo

    a = _A_ref(A_x, A_k_cache, A_v_cache, A_wq, A_wo)
    b = _B_ref(B_x, B_k_cache, B_v_cache, B_wq, B_wo)
    return jnp.concatenate([a, b], axis=-1)
```

```python
import jax
import jax.numpy as jnp
from jax import lax
import jax.experimental.pallas as pl
import jax.experimental.pallas.tpu as pltpu

B, SQ, D, H, SK, DH = 16, 80, 512, 32, 80, 128
M = B * SQ
C = (DH ** -0.5) * 1.4426950408889634
BF16 = jnp.bfloat16
F32 = jnp.float32

HG = 4
CB = 8
NC = B // CB
R = CB * SQ
SPB = H // HG
NSTEP = 2 * SPB
W = HG * DH

ORDER = (("Q", 1), ("K", 0), ("O", -2), ("V", -1), ("S", 0))


def _kernel(xa, ka, va, wqa, woa, xb, kb, vb, wqb, wob, out_hbm,
            x_buf, k_buf, v_buf, wq_buf, wo_buf, acc_ref, out_buf,
            sem_w, sem_h, sem_x, sem_o):
    one = pl.program_id(0) + 1
    refs_a = (ka, va, wqa, woa)
    refs_b = (kb, vb, wqb, wob)

    def group_copies(refs, g, sl):
        k_, v_, wq_, wo_ = refs
        off = g * W
        if not isinstance(off, int):
            off = pl.multiple_of(off, W)
        hh = g * HG
        return [
            pltpu.make_async_copy(wq_.at[:, pl.ds(off, W)], wq_buf.at[sl], sem_w.at[sl, 0]),
            pltpu.make_async_copy(k_.at[:, pl.ds(hh, HG)], k_buf.at[sl], sem_w.at[sl, 1]),
            pltpu.make_async_copy(v_.at[:, pl.ds(hh, HG)], v_buf.at[sl], sem_w.at[sl, 2]),
            pltpu.make_async_copy(wo_.at[pl.ds(off, W), :], wo_buf.at[sl], sem_w.at[sl, 3]),
        ]

    def head_copy(h, j, sem):
        off = h * DH
        if not isinstance(off, int):
            off = pl.multiple_of(off, DH)
        if j == 0:
            return pltpu.make_async_copy(wqa.at[:, pl.ds(off, DH)], wq_buf.at[0, :, pl.ds(off, DH)], sem)
        if j == 1:
            return pltpu.make_async_copy(ka.at[:, h], k_buf.at[0, :, h], sem)
        if j == 2:
            return pltpu.make_async_copy(va.at[:, h], v_buf.at[0, :, h], sem)
        return pltpu.make_async_copy(woa.at[pl.ds(off, DH), :], wo_buf.at[0, pl.ds(off, DH), :], sem)

    def start_group(gidx, sl):
        @pl.when(gidx < SPB)
        def _():
            for cp in group_copies(refs_a, gidx, sl):
                cp.start()

        @pl.when(jnp.logical_and(gidx >= SPB, gidx < NSTEP))
        def _():
            for cp in group_copies(refs_b, gidx - SPB, sl):
                cp.start()

    def wait_group(sl):
        for cp in group_copies(refs_a, 0, sl):
            cp.wait()

    def compute(slot, br, first, heads, write_out):
        slots = [(hi, c) for hi in range(len(heads)) for c in range(NC)]
        n = len(slots)
        q, sc, p, l, o = {}, {}, {}, {}, {}

        def hoff(hi):
            h = heads[hi]
            return h * DH if isinstance(h, int) else pl.multiple_of(h * DH, DH)

        def qproj(t):
            hi, c = slots[t]
            q[t] = jnp.dot(x_buf[br, c * R:(c + 1) * R, :],
                           wq_buf[slot, :, pl.ds(hoff(hi), DH)],
                           preferred_element_type=F32).astype(BF16)

        def qk(t):
            hi, c = slots[t]
            qt = q.pop(t)
            sc[t] = [lax.dot_general(qt[j * SQ:(j + 1) * SQ], k_buf[slot, c * CB + j, heads[hi]],
                                     (((1,), (1,)), ((), ())), preferred_element_type=F32)
                     for j in range(CB)]

        def softmax(t):
            p[t], l[t] = [], []
            for sj in sc.pop(t):
                m = jnp.max(sj, axis=-1, keepdims=True)
                pj = jnp.exp2((sj - m) * C)
                l[t].append(jnp.sum(pj, axis=-1, keepdims=True))
                p[t].append(pj.astype(BF16))

        def pv(t):
            hi, c = slots[t]
            pt, lt = p.pop(t), l.pop(t)
            outs = []
            for j in range(CB):
                oj = jnp.dot(pt[j], v_buf[slot, c * CB + j, heads[hi]], preferred_element_type=F32)
                r0 = pl.reciprocal(lt[j], approx=True)
                r1 = r0 * (2.0 - lt[j] * r0)
                outs.append((oj * r1).astype(BF16))
            o[t] = jnp.concatenate(outs, axis=0)

        def oproj(t):
            hi, c = slots[t]
            old = acc_ref[c * R:(c + 1) * R, :]
            if hi == 0:
                old = jnp.where(first, 0.0, old)
            new = old + jnp.dot(o.pop(t), wo_buf[slot, pl.ds(hoff(hi), DH), :],
                                preferred_element_type=F32)
            acc_ref[c * R:(c + 1) * R, :] = new
            if write_out and hi == len(heads) - 1:
                out_buf[br, c * R:(c + 1) * R, :] = new.astype(BF16)

        fns = dict(Q=qproj, K=qk, S=softmax, V=pv, O=oproj)
        lo = min(lag for _, lag in ORDER)
        hi_ = max(lag for _, lag in ORDER)
        for t in range(-hi_, n - lo):
            for st, lag in ORDER:
                if 0 <= t + lag < n:
                    fns[st](t + lag)

    xa_cp = pltpu.make_async_copy(xa, x_buf.at[0], sem_x.at[0])
    xb_cp = pltpu.make_async_copy(xb, x_buf.at[1], sem_x.at[1])
    xa_cp.start()
    head_copy(0, 0, sem_h.at[0, 0]).start()

    def start_head(h, carry):
        for j in range(1, 4):
            head_copy(h, j, sem_h.at[h, j]).start()

        @pl.when(h + 1 < HG)
        def _():
            head_copy(h + 1, 0, sem_h.at[h + 1, 0]).start()
        return carry
    lax.fori_loop(0, HG, start_head, 0)

    def start_g1(i, carry):
        for cp in group_copies(refs_a, 1, 1):
            cp.start()
        return carry
    lax.fori_loop(0, one, start_g1, 0)
    xa_cp.wait()

    def head_step(h, carry):
        for j in range(4):
            head_copy(0, j, sem_h.at[h, j]).wait()
        compute(0, 0, h == 0, [h], False)
        return carry
    lax.fori_loop(0, HG, head_step, 0)
    start_group(one + 1, 0)

    def step(s, carry):
        slot = s % 2
        br = s // SPB

        @pl.when(s == SPB)
        def _():
            xb_cp.wait()
        wait_group(slot)
        compute(slot, br, (s % SPB) == 0, list(range(HG)), True)
        start_group(s + 2, slot)

        @pl.when(s == 2)
        def _():
            xb_cp.start()

        @pl.when(s == SPB - 1)
        def _():
            pltpu.make_async_copy(out_buf.at[0], out_hbm.at[:, pl.ds(0, D)], sem_o.at[0]).start()
        return carry
    lax.fori_loop(1, NSTEP, step, 0)

    cpb = pltpu.make_async_copy(out_buf.at[1], out_hbm.at[:, pl.ds(D, D)], sem_o.at[1])
    cpb.start()
    pltpu.make_async_copy(out_buf.at[0], out_hbm.at[:, pl.ds(0, D)], sem_o.at[0]).wait()
    cpb.wait()


@jax.jit
def pallas_concat_heads__mha_block_cached__mha_block_cached__near_ridge_kernel(
    A_x: jax.Array,
    A_k_cache: jax.Array,
    A_v_cache: jax.Array,
    A_wq: jax.Array,
    A_wo: jax.Array,
    B_x: jax.Array,
    B_k_cache: jax.Array,
    B_v_cache: jax.Array,
    B_wq: jax.Array,
    B_wo: jax.Array,
):
    any_spec = pl.BlockSpec(memory_space=pl.ANY)
    out = pl.pallas_call(
        _kernel,
        grid=(1,),
        in_specs=[any_spec] * 10,
        out_specs=any_spec,
        out_shape=jax.ShapeDtypeStruct((M, 2 * D), BF16),
        scratch_shapes=[
            pltpu.VMEM((2, M, D), BF16),
            pltpu.VMEM((2, B, HG, SK, DH), BF16),
            pltpu.VMEM((2, B, HG, SK, DH), BF16),
            pltpu.VMEM((2, D, W), BF16),
            pltpu.VMEM((2, W, D), BF16),
            pltpu.VMEM((M, D), F32),
            pltpu.VMEM((2, M, D), BF16),
            pltpu.SemaphoreType.DMA((2, 4)),
            pltpu.SemaphoreType.DMA((HG, 4)),
            pltpu.SemaphoreType.DMA((2,)),
            pltpu.SemaphoreType.DMA((2,)),
        ],
        compiler_params=pltpu.CompilerParams(
            vmem_limit_bytes=100 * 1024 * 1024,
            disable_bounds_checks=True,
        ),
        name="mha2",
    )(A_x.reshape(M, D), A_k_cache, A_v_cache, A_wq, A_wo,
      B_x.reshape(M, D), B_k_cache, B_v_cache, B_wq, B_wo)
    return out.reshape(B, SQ, 2 * D)
```

```python
import jax
import jax.numpy as jnp
from jax import lax
import jax.experimental.pallas as pl
import jax.experimental.pallas.tpu as pltpu

B, SQ, D, H, SK, DH = 16, 80, 512, 32, 80, 128
M = B * SQ
C = (DH ** -0.5) * 1.4426950408889634
BF16 = jnp.bfloat16
F32 = jnp.float32

HG = 6
CB = 8
FG = 4
NA = (H - 2 * FG) // HG
NB = (H - 1) // HG
L = H - NB * HG
NJ = NA + NB
XC = 4
XR = M // XC
NQ1 = 2
assert 2 * FG + NA * HG == H and NB * HG + L == H and L <= HG

ORDER = (("Q", 1), ("K", 0), ("V", -1), ("O", -2), ("S", 0))


def _kernel(xa, ka, va, wqa, woa, xb, kb, vb, wqb, wob, out_hbm,
            x_buf, k_buf, v_buf, wq_buf, wo_buf, acc_ref, out_buf, q_buf,
            sem_w, sem_f, sem_x, sem_xb, sem_o):
    one = pl.program_id(0) + 1
    refs_a = (ka, va, wqa, woa)
    refs_b = (kb, vb, wqb, wob)

    def mo(v, m):
        return v if isinstance(v, int) else pl.multiple_of(v, m)

    def copies(refs, h0, nh, sl, sems):
        k_, v_, wq_, wo_ = refs
        so, w = mo(h0 * DH, DH), nh * DH
        return [
            pltpu.make_async_copy(wq_.at[:, pl.ds(so, w)], wq_buf.at[sl, :, pl.ds(0, w)], sems[0]),
            pltpu.make_async_copy(k_.at[:, pl.ds(h0, nh)], k_buf.at[sl, :, pl.ds(0, nh)], sems[1]),
            pltpu.make_async_copy(v_.at[:, pl.ds(h0, nh)], v_buf.at[sl, :, pl.ds(0, nh)], sems[2]),
            pltpu.make_async_copy(wo_.at[pl.ds(so, w), :], wo_buf.at[sl, pl.ds(0, w), :], sems[3]),
        ]

    def slot_of(j):
        return (j + 2) % 3

    def wsems(sl):
        return [sem_w.at[sl, i] for i in range(4)]

    def fcopies(g):
        return copies(refs_a, g * FG, FG, g, [sem_f.at[g, i] for i in range(4)])

    def x_copy(i):
        r = pl.ds(mo(i * XR, XR), XR)
        return pltpu.make_async_copy(xa.at[r], x_buf.at[0, r], sem_x.at[i])

    def start_group(j):
        sl = slot_of(j)

        @pl.when(j < NA)
        def _():
            for cp in copies(refs_a, 2 * FG + j * HG, HG, sl, wsems(sl)):
                cp.start()

        @pl.when(jnp.logical_and(j >= NA, j < NJ))
        def _():
            for cp in copies(refs_b, (j - NA) * HG, HG, sl, wsems(sl)):
                cp.start()

        @pl.when(j == NJ)
        def _():
            for cp in copies(refs_b, NB * HG, L, sl, wsems(sl)):
                cp.start()

    def wait_group(j, nh):
        sl = slot_of(j)
        for cp in copies(refs_a, 0, nh, sl, wsems(sl)):
            cp.wait()

    def compute(sl, br, first, nh, write_out, b0=0, nb=B, q0=None):
        nc = nb // CB
        rows_per = CB * SQ
        slots = [(hi, c) for hi in range(nh) for c in range(nc)]
        n = len(slots)
        q, sc, p, l, o = {}, {}, {}, {}, {}

        def rows(c):
            return pl.ds(mo((b0 + c * CB) * SQ, SQ), rows_per)

        def qproj(t):
            hi, c = slots[t]
            if q0 is not None:
                q[t] = q_buf[q0 + hi, rows(c), :]
            else:
                q[t] = jnp.dot(x_buf[br, rows(c), :], wq_buf[sl, :, hi * DH:(hi + 1) * DH],
                               preferred_element_type=F32).astype(BF16)

        def qk(t):
            hi, c = slots[t]
            qt = q.pop(t)
            sc[t] = [lax.dot_general(qt[j * SQ:(j + 1) * SQ], k_buf[sl, b0 + c * CB + j, hi],
                                     (((1,), (1,)), ((), ())), preferred_element_type=F32)
                     for j in range(CB)]

        def softmax(t):
            p[t], l[t] = [], []
            for sj in sc.pop(t):
                m = jnp.max(sj, axis=-1, keepdims=True)
                pj = jnp.exp2((sj - m) * C)
                l[t].append(jnp.sum(pj, axis=-1, keepdims=True))
                p[t].append(pj.astype(BF16))

        def pv(t):
            hi, c = slots[t]
            pt, lt = p.pop(t), l.pop(t)
            outs = []
            for j in range(CB):
                oj = jnp.dot(pt[j], v_buf[sl, b0 + c * CB + j, hi], preferred_element_type=F32)
                r0 = pl.reciprocal(lt[j], approx=True)
                r1 = r0 * (2.0 - lt[j] * r0)
                outs.append((oj * r1).astype(BF16))
            o[t] = jnp.concatenate(outs, axis=0)

        def oproj(t):
            hi, c = slots[t]
            old = acc_ref[rows(c), :]
            if hi == 0 and first is not None:
                old = jnp.where(first, 0.0, old)
            new = old + jnp.dot(o.pop(t), wo_buf[sl, hi * DH:(hi + 1) * DH, :],
                                preferred_element_type=F32)
            if write_out and hi == nh - 1:
                out_buf[br, rows(c), :] = new.astype(BF16)
            if not (write_out == "only" and hi == nh - 1):
                acc_ref[rows(c), :] = new

        fns = dict(Q=qproj, K=qk, S=softmax, V=pv, O=oproj)
        lo = min(lag for _, lag in ORDER)
        hi_ = max(lag for _, lag in ORDER)
        for t in range(-hi_, n - lo):
            for st, lag in ORDER:
                if 0 <= t + lag < n:
                    fns[st](t + lag)

    xb_cp = pltpu.make_async_copy(xb, x_buf.at[1], sem_xb.at[0])
    fcopies(0)[0].start()

    def start_x(i, c):
        x_copy(i).start()
        return c
    lax.fori_loop(0, XC, start_x, 0)

    def start_wq1(i, c):
        fcopies(1)[0].start()
        return c
    lax.fori_loop(0, one, start_wq1, 0)

    def start_kvo(g, c):
        for cp in fcopies(g)[1:]:
            cp.start()
        return c
    lax.fori_loop(0, 2, start_kvo, 0)

    def start_j(j, c):
        start_group(j)
        return c
    lax.fori_loop(0, one, start_j, 0)
    fcopies(0)[0].wait()

    def qdot(xr, g, h):
        return jnp.dot(xr, wq_buf[g, :, h * DH:(h + 1) * DH], preferred_element_type=F32).astype(BF16)

    def q_chunk(i, c):
        x_copy(i).wait()
        r = pl.ds(mo(i * XR, XR), XR)
        xr = x_buf[0, r, :]
        for h in range(FG):
            q_buf[h, r, :] = qdot(xr, 0, h)
        return c
    lax.fori_loop(0, NQ1, q_chunk, 0)
    for i in range(NQ1, XC):
        x_copy(i).wait()
    fcopies(1)[0].wait()
    xr = x_buf[0, NQ1 * XR:M, :]
    for h in range(FG):
        q_buf[h, NQ1 * XR:M, :] = qdot(xr, 0, h)
    xr = x_buf[0]
    for h in range(FG):
        q_buf[FG + h] = qdot(xr, 1, h)

    def first_attn(g, c):
        for cp in fcopies(g)[1:]:
            cp.wait()
        compute(g, 0, g == 0, FG, False, q0=g * FG)
        return c
    lax.fori_loop(0, 2, first_attn, 0)
    lax.fori_loop(1, one + 2, start_j, 0)

    def step(j, carry):
        br = (j >= NA).astype(jnp.int32)

        @pl.when(j == NA)
        def _():
            xb_cp.wait()
        wait_group(j, HG)
        compute(slot_of(j), br, j == NA, HG, True)
        start_group(j + 3)

        @pl.when(j == 0)
        def _():
            xb_cp.start()

        @pl.when(j == NA - 1)
        def _():
            pltpu.make_async_copy(out_buf.at[0], out_hbm.at[:, pl.ds(0, D)], sem_o.at[0]).start()
        return carry
    lax.fori_loop(0, NJ, step, 0)

    wait_group(NJ, L)
    hb = B // 2

    def out_half(c):
        r = pl.ds(mo(c * hb * SQ, hb * SQ), hb * SQ)
        return pltpu.make_async_copy(out_buf.at[1, r], out_hbm.at[r, pl.ds(D, D)], sem_o.at[1 + c])

    def last_step(c, carry):
        compute(slot_of(NJ), 1, None, L, "only", b0=c * hb, nb=hb)
        out_half(c).start()
        return carry
    lax.fori_loop(0, 2, last_step, 0)
    pltpu.make_async_copy(out_buf.at[0], out_hbm.at[:, pl.ds(0, D)], sem_o.at[0]).wait()
    out_half(0).wait()
    out_half(1).wait()


@jax.jit
def pallas_concat_heads__mha_block_cached__mha_block_cached__near_ridge_kernel(
    A_x: jax.Array,
    A_k_cache: jax.Array,
    A_v_cache: jax.Array,
    A_wq: jax.Array,
    A_wo: jax.Array,
    B_x: jax.Array,
    B_k_cache: jax.Array,
    B_v_cache: jax.Array,
    B_wq: jax.Array,
    B_wo: jax.Array,
):
    any_spec = pl.BlockSpec(memory_space=pl.ANY)
    out = pl.pallas_call(
        _kernel,
        grid=(1,),
        in_specs=[any_spec] * 10,
        out_specs=any_spec,
        out_shape=jax.ShapeDtypeStruct((M, 2 * D), BF16),
        scratch_shapes=[
            pltpu.VMEM((2, M, D), BF16),
            pltpu.VMEM((3, B, HG, SK, DH), BF16),
            pltpu.VMEM((3, B, HG, SK, DH), BF16),
            pltpu.VMEM((3, D, HG * DH), BF16),
            pltpu.VMEM((3, HG * DH, D), BF16),
            pltpu.VMEM((M, D), F32),
            pltpu.VMEM((2, M, D), BF16),
            pltpu.VMEM((2 * FG, M, DH), BF16),
            pltpu.SemaphoreType.DMA((3, 4)),
            pltpu.SemaphoreType.DMA((2, 4)),
            pltpu.SemaphoreType.DMA((XC,)),
            pltpu.SemaphoreType.DMA((1,)),
            pltpu.SemaphoreType.DMA((3,)),
        ],
        compiler_params=pltpu.CompilerParams(
            vmem_limit_bytes=100 * 1024 * 1024,
            disable_bounds_checks=True,
            disable_semaphore_checks=True,
        ),
        name="mha2",
    )(A_x.reshape(M, D), A_k_cache, A_v_cache, A_wq, A_wo,
      B_x.reshape(M, D), B_k_cache, B_v_cache, B_wq, B_wo)
    return out.reshape(B, SQ, 2 * D)
```

```python
import jax
import jax.numpy as jnp
from jax import lax
import jax.experimental.pallas as pl
import jax.experimental.pallas.tpu as pltpu

B, SQ, D, H, SK, DH = 16, 80, 512, 32, 80, 128
M = B * SQ
C = (DH ** -0.5) * 1.4426950408889634
BF16 = jnp.bfloat16
F32 = jnp.float32

HG = 6
CB = 8
FG = 4
NA = (H - 2 * FG) // HG
NB = (H - 1) // HG
L = H - NB * HG
NJ = NA + NB
XC = 4
XR = M // XC
NQ1 = 2
LCH = (4, 4, 4, 2, 2)
assert 2 * FG + NA * HG == H and NB * HG + L == H and L <= HG and sum(LCH) == B

ORDER = (("Q", 1), ("K", 0), ("V", -1), ("O", -2), ("S", 0))


def _kernel(xa, ka, va, wqa, woa, xb, kb, vb, wqb, wob, out_hbm,
            x_buf, k_buf, v_buf, wq_buf, wo_buf, acc_ref, out_buf, q_buf,
            sem_w, sem_f, sem_x, sem_xb, sem_o):
    one = pl.program_id(0) + 1
    refs_a = (ka, va, wqa, woa)
    refs_b = (kb, vb, wqb, wob)

    def mo(v, m):
        return v if isinstance(v, int) else pl.multiple_of(v, m)

    def copies(refs, h0, nh, sl, sems):
        k_, v_, wq_, wo_ = refs
        so, w = mo(h0 * DH, DH), nh * DH
        return [
            pltpu.make_async_copy(wq_.at[:, pl.ds(so, w)], wq_buf.at[sl, :, pl.ds(0, w)], sems[0]),
            pltpu.make_async_copy(k_.at[:, pl.ds(h0, nh)], k_buf.at[sl, :, pl.ds(0, nh)], sems[1]),
            pltpu.make_async_copy(v_.at[:, pl.ds(h0, nh)], v_buf.at[sl, :, pl.ds(0, nh)], sems[2]),
            pltpu.make_async_copy(wo_.at[pl.ds(so, w), :], wo_buf.at[sl, pl.ds(0, w), :], sems[3]),
        ]

    def wsems(sl):
        return [sem_w.at[sl, i] for i in range(4)]

    def fcopies(g):
        return copies(refs_a, g * FG, FG, g, [sem_f.at[g, i] for i in range(4)])

    def x_copy(i):
        r = pl.ds(mo(i * XR, XR), XR)
        return pltpu.make_async_copy(xa.at[r], x_buf.at[0, r], sem_x.at[i])

    def start_group(j, sl):
        @pl.when(j < NA)
        def _():
            for cp in copies(refs_a, 2 * FG + j * HG, HG, sl, wsems(sl)):
                cp.start()

        @pl.when(jnp.logical_and(j >= NA, j < NJ))
        def _():
            for cp in copies(refs_b, (j - NA) * HG, HG, sl, wsems(sl)):
                cp.start()

        @pl.when(j == NJ)
        def _():
            for cp in copies(refs_b, NB * HG, L, sl, wsems(sl)):
                cp.start()

    def wait_group(sl, nh):
        for cp in copies(refs_a, 0, nh, sl, wsems(sl)):
            cp.wait()

    def compute(sl, br, first, slots, write_out, q0=None, after_out=None):
        n = len(slots)
        hmin = min(s[0] for s in slots)
        hmax = max(s[0] for s in slots)
        q, sc, p, l, o = {}, {}, {}, {}, {}

        def rows(t):
            _, b0, nb = slots[t]
            return slice(b0 * SQ, (b0 + nb) * SQ)

        def qproj(t):
            hi = slots[t][0]
            if q0 is not None:
                q[t] = q_buf[q0 + hi, rows(t), :]
            else:
                q[t] = jnp.dot(x_buf[br, rows(t), :], wq_buf[sl, :, hi * DH:(hi + 1) * DH],
                               preferred_element_type=F32).astype(BF16)

        def qk(t):
            hi, b0, nb = slots[t]
            qt = q.pop(t)
            sc[t] = [lax.dot_general(qt[j * SQ:(j + 1) * SQ], k_buf[sl, b0 + j, hi],
                                     (((1,), (1,)), ((), ())), preferred_element_type=F32)
                     for j in range(nb)]

        def softmax(t):
            p[t], l[t] = [], []
            for sj in sc.pop(t):
                m = jnp.max(sj, axis=-1, keepdims=True)
                pj = jnp.exp2((sj - m) * C)
                l[t].append(jnp.sum(pj, axis=-1, keepdims=True))
                p[t].append(pj.astype(BF16))

        def pv(t):
            hi, b0, nb = slots[t]
            pt, lt = p.pop(t), l.pop(t)
            outs = []
            for j in range(nb):
                oj = jnp.dot(pt[j], v_buf[sl, b0 + j, hi], preferred_element_type=F32)
                r0 = pl.reciprocal(lt[j], approx=True)
                r1 = r0 * (2.0 - lt[j] * r0)
                outs.append((oj * r1).astype(BF16))
            o[t] = jnp.concatenate(outs, axis=0)

        def oproj(t):
            hi = slots[t][0]
            old = acc_ref[rows(t), :]
            if hi == hmin and first is not None:
                old = jnp.where(first, 0.0, old)
            new = old + jnp.dot(o.pop(t), wo_buf[sl, hi * DH:(hi + 1) * DH, :],
                                preferred_element_type=F32)
            if write_out and hi == hmax:
                out_buf[br, rows(t), :] = new.astype(BF16)
                if after_out is not None:
                    after_out(t)
            if not (write_out == "only" and hi == hmax):
                acc_ref[rows(t), :] = new

        fns = dict(Q=qproj, K=qk, S=softmax, V=pv, O=oproj)
        lo = min(lag for _, lag in ORDER)
        hi_ = max(lag for _, lag in ORDER)
        for t in range(-hi_, n - lo):
            for st, lag in ORDER:
                if 0 <= t + lag < n:
                    fns[st](t + lag)

    def head_major(nh):
        return [(hi, c * CB, CB) for hi in range(nh) for c in range(B // CB)]

    xb_cp = pltpu.make_async_copy(xb, x_buf.at[1], sem_xb.at[0])
    fcopies(0)[0].start()

    def start_x(i, c):
        x_copy(i).start()
        return c
    lax.fori_loop(0, XC, start_x, 0)

    def start_wq1(i, c):
        fcopies(1)[0].start()
        return c
    lax.fori_loop(0, one, start_wq1, 0)

    def start_kvo(g, c):
        for cp in fcopies(g)[1:]:
            cp.start()
        return c
    lax.fori_loop(0, 2, start_kvo, 0)

    def start_g0(j, c):
        start_group(j, 2)
        return c
    lax.fori_loop(0, one, start_g0, 0)
    fcopies(0)[0].wait()

    def qdot(xr, g, h):
        return jnp.dot(xr, wq_buf[g, :, h * DH:(h + 1) * DH], preferred_element_type=F32).astype(BF16)

    def q_chunk(i, c):
        x_copy(i).wait()
        r = pl.ds(mo(i * XR, XR), XR)
        xr = x_buf[0, r, :]
        for h in range(FG):
            q_buf[h, r, :] = qdot(xr, 0, h)
        return c
    lax.fori_loop(0, NQ1, q_chunk, 0)
    for i in range(NQ1, XC):
        x_copy(i).wait()
    fcopies(1)[0].wait()
    xr = x_buf[0, NQ1 * XR:M, :]
    for h in range(FG):
        q_buf[h, NQ1 * XR:M, :] = qdot(xr, 0, h)
    xr = x_buf[0]
    for h in range(FG):
        q_buf[FG + h] = qdot(xr, 1, h)

    def first_attn(g, c):
        for cp in fcopies(g)[1:]:
            cp.wait()
        compute(g, 0, g == 0, head_major(FG), False, q0=g * FG)
        start_group(g + 1, g)
        return c
    lax.fori_loop(0, 2, first_attn, 0)

    def step(j, sl):
        br = (j >= NA).astype(jnp.int32)

        @pl.when(j == NA)
        def _():
            xb_cp.wait()
        wait_group(sl, HG)
        compute(sl, br, j == NA, head_major(HG), True)
        start_group(j + 3, sl)

        @pl.when(j == 0)
        def _():
            xb_cp.start()

        @pl.when(j == NA - 1)
        def _():
            pltpu.make_async_copy(out_buf.at[0], out_hbm.at[:, pl.ds(0, D)], sem_o.at[0]).start()
        return jnp.where(sl == 2, 0, sl + 1)
    lax.fori_loop(0, NJ, step, 2 * one)

    lsl = (NJ + 2) % 3
    wait_group(lsl, L)
    slots, b0 = [], 0
    for nb in LCH:
        slots += [(hi, b0, nb) for hi in range(L)]
        b0 += nb

    def out_part(t):
        _, b0, nb = slots[t]
        r = pl.ds(b0 * SQ, nb * SQ)
        return pltpu.make_async_copy(out_buf.at[1, r], out_hbm.at[r, pl.ds(D, D)],
                                     sem_o.at[1 + t // L])

    compute(lsl, 1, None, slots, "only", after_out=lambda t: out_part(t).start())
    pltpu.make_async_copy(out_buf.at[0], out_hbm.at[:, pl.ds(0, D)], sem_o.at[0]).wait()
    for t in range(L - 1, len(slots), L):
        out_part(t).wait()


@jax.jit
def pallas_concat_heads__mha_block_cached__mha_block_cached__near_ridge_kernel(
    A_x: jax.Array,
    A_k_cache: jax.Array,
    A_v_cache: jax.Array,
    A_wq: jax.Array,
    A_wo: jax.Array,
    B_x: jax.Array,
    B_k_cache: jax.Array,
    B_v_cache: jax.Array,
    B_wq: jax.Array,
    B_wo: jax.Array,
):
    any_spec = pl.BlockSpec(memory_space=pl.ANY)
    out = pl.pallas_call(
        _kernel,
        grid=(1,),
        in_specs=[any_spec] * 10,
        out_specs=any_spec,
        out_shape=jax.ShapeDtypeStruct((M, 2 * D), BF16),
        scratch_shapes=[
            pltpu.VMEM((2, M, D), BF16),
            pltpu.VMEM((3, B, HG, SK, DH), BF16),
            pltpu.VMEM((3, B, HG, SK, DH), BF16),
            pltpu.VMEM((3, D, HG * DH), BF16),
            pltpu.VMEM((3, HG * DH, D), BF16),
            pltpu.VMEM((M, D), F32),
            pltpu.VMEM((2, M, D), BF16),
            pltpu.VMEM((2 * FG, M, DH), BF16),
            pltpu.SemaphoreType.DMA((3, 4)),
            pltpu.SemaphoreType.DMA((2, 4)),
            pltpu.SemaphoreType.DMA((XC,)),
            pltpu.SemaphoreType.DMA((1,)),
            pltpu.SemaphoreType.DMA((1 + len(LCH),)),
        ],
        compiler_params=pltpu.CompilerParams(
            vmem_limit_bytes=100 * 1024 * 1024,
            disable_bounds_checks=True,
            disable_semaphore_checks=True,
        ),
        name="mha2",
    )(A_x.reshape(M, D), A_k_cache, A_v_cache, A_wq, A_wo,
      B_x.reshape(M, D), B_k_cache, B_v_cache, B_wq, B_wo)
    return out.reshape(B, SQ, 2 * D)
```

```python
import jax
import jax.numpy as jnp
from jax import lax
import jax.experimental.pallas as pl
import jax.experimental.pallas.tpu as pltpu

B, SQ, D, H, SK, DH = 16, 80, 512, 32, 80, 128
M = B * SQ
C = (DH ** -0.5) * 1.4426950408889634
BF16 = jnp.bfloat16
F32 = jnp.float32

HG = 6
CB = 8
FG = 4
NA = (H - 2 * FG) // HG
NB = (H - 1) // HG
L = H - NB * HG
NJ = NA + NB
XC = 4
XR = M // XC
LCH = (4, 4, 4, 2, 2)
assert 2 * FG + NA * HG == H and NB * HG + L == H and L <= HG and sum(LCH) == B

ORDER = (("Q", 1), ("K", 0), ("V", -1), ("O", -2), ("S", 0))


def _kernel(xa, ka, va, wqa, woa, xb, kb, vb, wqb, wob, out_hbm,
            x_buf, k_buf, v_buf, wq_buf, wo_buf, acc_ref, out_buf, q_buf,
            sem_w, sem_f, sem_x, sem_p, sem_xb, sem_o):
    one = pl.program_id(0) + 1
    refs_a = (ka, va, wqa, woa)
    refs_b = (kb, vb, wqb, wob)

    def mo(v, m):
        return v if isinstance(v, int) else pl.multiple_of(v, m)

    def once(fn):
        def body(_, c):
            fn()
            return c
        lax.fori_loop(0, one, body, 0)

    def copies(refs, h0, nh, sl, sems):
        k_, v_, wq_, wo_ = refs
        so, w = mo(h0 * DH, DH), nh * DH
        return [
            pltpu.make_async_copy(wq_.at[:, pl.ds(so, w)], wq_buf.at[sl, :, pl.ds(0, w)], sems[0]),
            pltpu.make_async_copy(k_.at[:, pl.ds(h0, nh)], k_buf.at[sl, :, pl.ds(0, nh)], sems[1]),
            pltpu.make_async_copy(v_.at[:, pl.ds(h0, nh)], v_buf.at[sl, :, pl.ds(0, nh)], sems[2]),
            pltpu.make_async_copy(wo_.at[pl.ds(so, w), :], wo_buf.at[sl, pl.ds(0, w), :], sems[3]),
        ]

    def wsems(sl):
        return [sem_w.at[sl, i] for i in range(4)]

    def kvo_copies(g):
        return copies(refs_a, g * FG, FG, g, [sem_f.at[g, i] for i in range(4)])[1:]

    def wq1_copy():
        return copies(refs_a, FG, FG, 1, [sem_f.at[1, i] for i in range(4)])[0]

    def wq_pair(i):
        cols = pl.ds(mo(i * 2 * DH, 2 * DH), 2 * DH)
        return pltpu.make_async_copy(wqa.at[:, cols], wq_buf.at[0, :, cols], sem_p.at[i])

    def x_copy(i):
        r = pl.ds(mo(i * XR, XR), XR)
        return pltpu.make_async_copy(xa.at[r], x_buf.at[0, r], sem_x.at[i])

    xb_cp = pltpu.make_async_copy(xb, x_buf.at[1], sem_xb.at[0])

    def start_group(j, sl):
        @pl.when(j < NA)
        def _():
            for cp in copies(refs_a, 2 * FG + j * HG, HG, sl, wsems(sl)):
                cp.start()

        @pl.when(jnp.logical_and(j >= NA, j < NJ))
        def _():
            for cp in copies(refs_b, (j - NA) * HG, HG, sl, wsems(sl)):
                cp.start()

        @pl.when(j == NJ)
        def _():
            for cp in copies(refs_b, NB * HG, L, sl, wsems(sl)):
                cp.start()

    def wait_group(sl, nh):
        for cp in copies(refs_a, 0, nh, sl, wsems(sl)):
            cp.wait()

    def compute(sl, br, first, slots, write_out, q0=None, after_out=None):
        n = len(slots)
        hmin = min(s[0] for s in slots)
        hmax = max(s[0] for s in slots)
        q, sc, p, l, o = {}, {}, {}, {}, {}

        def rows(t):
            _, b0, nb = slots[t]
            return slice(b0 * SQ, (b0 + nb) * SQ)

        def qproj(t):
            hi = slots[t][0]
            if q0 is not None:
                q[t] = q_buf[q0 + hi, rows(t), :]
            else:
                q[t] = jnp.dot(x_buf[br, rows(t), :], wq_buf[sl, :, hi * DH:(hi + 1) * DH],
                               preferred_element_type=F32).astype(BF16)

        def qk(t):
            hi, b0, nb = slots[t]
            qt = q.pop(t)
            sc[t] = [lax.dot_general(qt[j * SQ:(j + 1) * SQ], k_buf[sl, b0 + j, hi],
                                     (((1,), (1,)), ((), ())), preferred_element_type=F32)
                     for j in range(nb)]

        def softmax(t):
            p[t], l[t] = [], []
            for sj in sc.pop(t):
                m = jnp.max(sj, axis=-1, keepdims=True)
                pj = jnp.exp2((sj - m) * C)
                l[t].append(jnp.sum(pj, axis=-1, keepdims=True))
                p[t].append(pj.astype(BF16))

        def pv(t):
            hi, b0, nb = slots[t]
            pt, lt = p.pop(t), l.pop(t)
            outs = []
            for j in range(nb):
                oj = jnp.dot(pt[j], v_buf[sl, b0 + j, hi], preferred_element_type=F32)
                r0 = pl.reciprocal(lt[j], approx=True)
                r1 = r0 * (2.0 - lt[j] * r0)
                outs.append((oj * r1).astype(BF16))
            o[t] = jnp.concatenate(outs, axis=0)

        def oproj(t):
            hi = slots[t][0]
            old = acc_ref[rows(t), :]
            if hi == hmin and first is not None:
                old = jnp.where(first, 0.0, old)
            new = old + jnp.dot(o.pop(t), wo_buf[sl, hi * DH:(hi + 1) * DH, :],
                                preferred_element_type=F32)
            if write_out and hi == hmax:
                out_buf[br, rows(t), :] = new.astype(BF16)
                if after_out is not None:
                    after_out(t)
            if not (write_out == "only" and hi == hmax):
                acc_ref[rows(t), :] = new

        fns = dict(Q=qproj, K=qk, S=softmax, V=pv, O=oproj)
        lo = min(lag for _, lag in ORDER)
        hi_ = max(lag for _, lag in ORDER)
        for t in range(-hi_, n - lo):
            for st, lag in ORDER:
                if 0 <= t + lag < n:
                    fns[st](t + lag)

    def head_major(nh):
        return [(hi, c * CB, CB) for hi in range(nh) for c in range(B // CB)]

    def qdot(xr, g, cols):
        return jnp.dot(xr, wq_buf[g, :, cols], preferred_element_type=F32).astype(BF16)

    def head_cols(h):
        return pl.ds(mo(h * DH, DH), DH)

    def first_phase():
        wq_pair(0).start()
        once(lambda: x_copy(0).start())
        once(lambda: wq_pair(1).start())

        def start_x(i, c):
            x_copy(i).start()
            return c
        lax.fori_loop(1, XC, start_x, 0)
        once(lambda: wq1_copy().start())

        def start_kvo(g, c):
            for cp in kvo_copies(g):
                cp.start()
            return c
        lax.fori_loop(0, 2, start_kvo, 0)
        once(lambda: start_group(one - 1, 2))

        x_copy(0).wait()

        def q_pair(i, c):
            wq_pair(i).wait()
            xr = x_buf[0, 0:XR, :]
            for hh in range(2):
                q_buf[2 * i + hh, 0:XR, :] = qdot(xr, 0, head_cols(2 * i + hh))
            return c
        lax.fori_loop(0, FG // 2, q_pair, 0)
        x_copy(1).wait()
        x_copy(2).wait()

        def q_mid():
            xr = x_buf[0, XR:3 * XR, :]
            for h in range(FG):
                q_buf[h, XR:3 * XR, :] = qdot(xr, 0, head_cols(h))
        once(q_mid)
        x_copy(3).wait()
        wq1_copy().wait()
        xr = x_buf[0, 3 * XR:M, :]
        for h in range(FG):
            q_buf[h, 3 * XR:M, :] = qdot(xr, 0, head_cols(h))
        xr = x_buf[0]
        for h in range(FG):
            q_buf[FG + h] = qdot(xr, 1, head_cols(h))

        def first_attn(g, c):
            for cp in kvo_copies(g):
                cp.wait()
            compute(g, 0, g == 0, head_major(FG), False, q0=g * FG)
            start_group(g + 1, g)
            return c
        lax.fori_loop(0, 2, first_attn, 0)

    def main_step(j, sl):
        br = (j >= NA).astype(jnp.int32)

        @pl.when(j == NA)
        def _():
            xb_cp.wait()
        wait_group(sl, HG)
        compute(sl, br, j == NA, head_major(HG), True)
        start_group(j + 3, sl)

        @pl.when(j == 0)
        def _():
            xb_cp.start()

        @pl.when(j == NA - 1)
        def _():
            pltpu.make_async_copy(out_buf.at[0], out_hbm.at[:, pl.ds(0, D)], sem_o.at[0]).start()

    def last_phase():
        lsl = (NJ + 2) % 3
        wait_group(lsl, L)
        slots, b0 = [], 0
        for nb in LCH:
            slots += [(hi, b0, nb) for hi in range(L)]
            b0 += nb

        def out_part(t):
            _, b0, nb = slots[t]
            r = pl.ds(b0 * SQ, nb * SQ)
            return pltpu.make_async_copy(out_buf.at[1, r], out_hbm.at[r, pl.ds(D, D)],
                                         sem_o.at[1 + t // L])

        compute(lsl, 1, None, slots, "only", after_out=lambda t: out_part(t).start())
        pltpu.make_async_copy(out_buf.at[0], out_hbm.at[:, pl.ds(0, D)], sem_o.at[0]).wait()
        for t in range(L - 1, len(slots), L):
            out_part(t).wait()

    def phase(s, sl):
        pl.when(jnp.logical_and(s >= 1, s <= NJ))(lambda: main_step(s - 1, sl))
        pl.when(s == NJ + 1)(last_phase)
        pl.when(s == 0)(first_phase)
        return jnp.where(jnp.logical_or(s == 0, sl == 0), jnp.where(s == 0, 2, 1),
                         jnp.where(sl == 1, 2, 0))
    lax.fori_loop(0, NJ + 2, phase, 2 * one)


@jax.jit
def pallas_concat_heads__mha_block_cached__mha_block_cached__near_ridge_kernel(
    A_x: jax.Array,
    A_k_cache: jax.Array,
    A_v_cache: jax.Array,
    A_wq: jax.Array,
    A_wo: jax.Array,
    B_x: jax.Array,
    B_k_cache: jax.Array,
    B_v_cache: jax.Array,
    B_wq: jax.Array,
    B_wo: jax.Array,
):
    any_spec = pl.BlockSpec(memory_space=pl.ANY)
    out = pl.pallas_call(
        _kernel,
        grid=(1,),
        in_specs=[any_spec] * 10,
        out_specs=any_spec,
        out_shape=jax.ShapeDtypeStruct((M, 2 * D), BF16),
        scratch_shapes=[
            pltpu.VMEM((2, M, D), BF16),
            pltpu.VMEM((3, B, HG, SK, DH), BF16),
            pltpu.VMEM((3, B, HG, SK, DH), BF16),
            pltpu.VMEM((3, D, HG * DH), BF16),
            pltpu.VMEM((3, HG * DH, D), BF16),
            pltpu.VMEM((M, D), F32),
            pltpu.VMEM((2, M, D), BF16),
            pltpu.VMEM((2 * FG, M, DH), BF16),
            pltpu.SemaphoreType.DMA((3, 4)),
            pltpu.SemaphoreType.DMA((2, 4)),
            pltpu.SemaphoreType.DMA((XC,)),
            pltpu.SemaphoreType.DMA((FG // 2,)),
            pltpu.SemaphoreType.DMA((1,)),
            pltpu.SemaphoreType.DMA((1 + len(LCH),)),
        ],
        compiler_params=pltpu.CompilerParams(
            vmem_limit_bytes=100 * 1024 * 1024,
            disable_bounds_checks=True,
            disable_semaphore_checks=True,
        ),
        name="mha2",
    )(A_x.reshape(M, D), A_k_cache, A_v_cache, A_wq, A_wo,
      B_x.reshape(M, D), B_k_cache, B_v_cache, B_wq, B_wo)
    return out.reshape(B, SQ, 2 * D)
```

```python
import jax
import jax.numpy as jnp
from jax import lax
import jax.experimental.pallas as pl
import jax.experimental.pallas.tpu as pltpu

B, SQ, D, H, SK, DH = 16, 80, 512, 32, 80, 128
M = B * SQ
C = (DH ** -0.5) * 1.4426950408889634
BF16 = jnp.bfloat16
F32 = jnp.float32

HG = 6
CB = 8
FG = 4
NA = (H - 2 * FG) // HG
NB = (H - 1) // HG
L = H - NB * HG
NJ = NA + NB
XC = 4
XR = M // XC
LCH = (4, 4, 4, 2, 2)
assert 2 * FG + NA * HG == H and NB * HG + L == H and L <= HG and sum(LCH) == B

LAG = dict(Q=1, K=0, S=0, V=-1, O=-2)
MAIN_ORDER = "VKOQS"
EDGE_ORDER = "QKVOS"


def _kernel(xa, ka, va, wqa, woa, xb, kb, vb, wqb, wob, out_hbm,
            x_buf, k_buf, v_buf, wq_buf, wo_buf, acc_ref, out_buf, q_buf,
            sem_w, sem_f, sem_x, sem_p, sem_xb, sem_o):
    one = pl.program_id(0) + 1
    refs_a = (ka, va, wqa, woa)
    refs_b = (kb, vb, wqb, wob)

    def mo(v, m):
        return v if isinstance(v, int) else pl.multiple_of(v, m)

    def once(fn):
        def body(_, c):
            fn()
            return c
        lax.fori_loop(0, one, body, 0)

    def copies(refs, h0, nh, sl, sems):
        k_, v_, wq_, wo_ = refs
        so, w = mo(h0 * DH, DH), nh * DH
        return [
            pltpu.make_async_copy(wq_.at[:, pl.ds(so, w)], wq_buf.at[sl, :, pl.ds(0, w)], sems[0]),
            pltpu.make_async_copy(k_.at[:, pl.ds(h0, nh)], k_buf.at[sl, :, pl.ds(0, nh)], sems[1]),
            pltpu.make_async_copy(v_.at[:, pl.ds(h0, nh)], v_buf.at[sl, :, pl.ds(0, nh)], sems[2]),
            pltpu.make_async_copy(wo_.at[pl.ds(so, w), :], wo_buf.at[sl, pl.ds(0, w), :], sems[3]),
        ]

    def wsems(sl):
        return [sem_w.at[sl, i] for i in range(4)]

    def kvo_copies(g):
        return copies(refs_a, g * FG, FG, g, [sem_f.at[g, i] for i in range(4)])[1:]

    def wq1_copy():
        return copies(refs_a, FG, FG, 1, [sem_f.at[1, i] for i in range(4)])[0]

    def wq_pair(i):
        cols = pl.ds(mo(i * 2 * DH, 2 * DH), 2 * DH)
        return pltpu.make_async_copy(wqa.at[:, cols], wq_buf.at[0, :, cols], sem_p.at[i])

    def x_copy(i):
        r = pl.ds(mo(i * XR, XR), XR)
        return pltpu.make_async_copy(xa.at[r], x_buf.at[0, r], sem_x.at[i])

    xb_cp = pltpu.make_async_copy(xb, x_buf.at[1], sem_xb.at[0])

    def start_group(j, sl):
        @pl.when(j < NA)
        def _():
            for cp in copies(refs_a, 2 * FG + j * HG, HG, sl, wsems(sl)):
                cp.start()

        @pl.when(jnp.logical_and(j >= NA, j < NJ))
        def _():
            for cp in copies(refs_b, (j - NA) * HG, HG, sl, wsems(sl)):
                cp.start()

        @pl.when(j == NJ)
        def _():
            for cp in copies(refs_b, NB * HG, L, sl, wsems(sl)):
                cp.start()

    def wait_group(sl, nh):
        for cp in copies(refs_a, 0, nh, sl, wsems(sl)):
            cp.wait()

    def compute(order, sl, br, first, slots, write_out, q0=None, after_out=None):
        n = len(slots)
        hmin = min(s[0] for s in slots)
        hmax = max(s[0] for s in slots)
        q, sc, p, l, o = {}, {}, {}, {}, {}

        def rows(t):
            _, b0, nb = slots[t]
            return slice(b0 * SQ, (b0 + nb) * SQ)

        def qproj(t):
            hi = slots[t][0]
            if q0 is not None:
                q[t] = q_buf[q0 + hi, rows(t), :]
            else:
                q[t] = jnp.dot(x_buf[br, rows(t), :], wq_buf[sl, :, hi * DH:(hi + 1) * DH],
                               preferred_element_type=F32).astype(BF16)

        def qk(t):
            hi, b0, nb = slots[t]
            qt = q.pop(t)
            sc[t] = [lax.dot_general(qt[j * SQ:(j + 1) * SQ], k_buf[sl, b0 + j, hi],
                                     (((1,), (1,)), ((), ())), preferred_element_type=F32)
                     for j in range(nb)]

        def softmax(t):
            p[t], l[t] = [], []
            for sj in sc.pop(t):
                m = jnp.max(sj, axis=-1, keepdims=True)
                pj = jnp.exp2((sj - m) * C)
                l[t].append(jnp.sum(pj, axis=-1, keepdims=True))
                p[t].append(pj.astype(BF16))

        def pv(t):
            hi, b0, nb = slots[t]
            pt, lt = p.pop(t), l.pop(t)
            outs = []
            for j in range(nb):
                oj = jnp.dot(pt[j], v_buf[sl, b0 + j, hi], preferred_element_type=F32)
                r0 = pl.reciprocal(lt[j], approx=True)
                r1 = r0 * (2.0 - lt[j] * r0)
                outs.append((oj * r1).astype(BF16))
            o[t] = jnp.concatenate(outs, axis=0)

        def oproj(t):
            hi = slots[t][0]
            old = acc_ref[rows(t), :]
            if hi == hmin and first is not None:
                old = jnp.where(first, 0.0, old)
            new = old + jnp.dot(o.pop(t), wo_buf[sl, hi * DH:(hi + 1) * DH, :],
                                preferred_element_type=F32)
            if write_out and hi == hmax:
                out_buf[br, rows(t), :] = new.astype(BF16)
                if after_out is not None:
                    after_out(t)
            if not (write_out == "only" and hi == hmax):
                acc_ref[rows(t), :] = new

        fns = dict(Q=qproj, K=qk, S=softmax, V=pv, O=oproj)
        for t in range(-max(LAG.values()), n - min(LAG.values())):
            for st in order:
                if 0 <= t + LAG[st] < n:
                    fns[st](t + LAG[st])

    def head_major(nh):
        return [(hi, c * CB, CB) for hi in range(nh) for c in range(B // CB)]

    def qdot(xr, g, cols):
        return jnp.dot(xr, wq_buf[g, :, cols], preferred_element_type=F32).astype(BF16)

    def head_cols(h):
        return pl.ds(mo(h * DH, DH), DH)

    def first_phase():
        wq_pair(0).start()
        once(lambda: x_copy(0).start())
        once(lambda: wq_pair(1).start())

        def start_x(i, c):
            x_copy(i).start()
            return c
        lax.fori_loop(1, XC, start_x, 0)
        once(lambda: wq1_copy().start())

        def start_kvo(g, c):
            for cp in kvo_copies(g):
                cp.start()
            return c
        lax.fori_loop(0, 2, start_kvo, 0)
        once(lambda: start_group(one - 1, 2))

        x_copy(0).wait()

        def q_pair(i, c):
            wq_pair(i).wait()
            xr = x_buf[0, 0:XR, :]
            for hh in range(2):
                q_buf[2 * i + hh, 0:XR, :] = qdot(xr, 0, head_cols(2 * i + hh))
            return c
        lax.fori_loop(0, FG // 2, q_pair, 0)
        x_copy(1).wait()
        x_copy(2).wait()

        def q_mid():
            xr = x_buf[0, XR:3 * XR, :]
            for h in range(FG):
                q_buf[h, XR:3 * XR, :] = qdot(xr, 0, head_cols(h))
        once(q_mid)
        x_copy(3).wait()
        wq1_copy().wait()
        xr = x_buf[0, 3 * XR:M, :]
        for h in range(FG):
            q_buf[h, 3 * XR:M, :] = qdot(xr, 0, head_cols(h))
        xr = x_buf[0]
        for h in range(FG):
            q_buf[FG + h] = qdot(xr, 1, head_cols(h))

        def first_attn(g, c):
            for cp in kvo_copies(g):
                cp.wait()
            compute(EDGE_ORDER, g, 0, g == 0, head_major(FG), False, q0=g * FG)
            start_group(g + 1, g)
            return c
        lax.fori_loop(0, 2, first_attn, 0)

    def main_step(j, sl):
        br = (j >= NA).astype(jnp.int32)

        @pl.when(j == NA)
        def _():
            xb_cp.wait()
        wait_group(sl, HG)
        compute(MAIN_ORDER, sl, br, j == NA, head_major(HG), True)
        start_group(j + 3, sl)

        @pl.when(j == 0)
        def _():
            xb_cp.start()

        @pl.when(j == NA - 1)
        def _():
            pltpu.make_async_copy(out_buf.at[0], out_hbm.at[:, pl.ds(0, D)], sem_o.at[0]).start()

    def last_phase():
        lsl = (NJ + 2) % 3
        wait_group(lsl, L)
        slots, b0 = [], 0
        for nb in LCH:
            slots += [(hi, b0, nb) for hi in range(L)]
            b0 += nb

        def out_part(t):
            _, b0, nb = slots[t]
            r = pl.ds(b0 * SQ, nb * SQ)
            return pltpu.make_async_copy(out_buf.at[1, r], out_hbm.at[r, pl.ds(D, D)],
                                         sem_o.at[1 + t // L])

        compute(EDGE_ORDER, lsl, 1, None, slots, "only", after_out=lambda t: out_part(t).start())
        pltpu.make_async_copy(out_buf.at[0], out_hbm.at[:, pl.ds(0, D)], sem_o.at[0]).wait()
        for t in range(L - 1, len(slots), L):
            out_part(t).wait()

    def phase(s, sl):
        pl.when(jnp.logical_and(s >= 1, s <= NJ))(lambda: main_step(s - 1, sl))
        pl.when(s == NJ + 1)(last_phase)
        pl.when(s == 0)(first_phase)
        return jnp.where(s == 0, 2, jnp.where(sl == 2, 0, sl + 1))
    lax.fori_loop(0, NJ + 2, phase, 2 * one)


@jax.jit
def pallas_concat_heads__mha_block_cached__mha_block_cached__near_ridge_kernel(
    A_x: jax.Array,
    A_k_cache: jax.Array,
    A_v_cache: jax.Array,
    A_wq: jax.Array,
    A_wo: jax.Array,
    B_x: jax.Array,
    B_k_cache: jax.Array,
    B_v_cache: jax.Array,
    B_wq: jax.Array,
    B_wo: jax.Array,
):
    any_spec = pl.BlockSpec(memory_space=pl.ANY)
    out = pl.pallas_call(
        _kernel,
        grid=(1,),
        in_specs=[any_spec] * 10,
        out_specs=any_spec,
        out_shape=jax.ShapeDtypeStruct((M, 2 * D), BF16),
        scratch_shapes=[
            pltpu.VMEM((2, M, D), BF16),
            pltpu.VMEM((3, B, HG, SK, DH), BF16),
            pltpu.VMEM((3, B, HG, SK, DH), BF16),
            pltpu.VMEM((3, D, HG * DH), BF16),
            pltpu.VMEM((3, HG * DH, D), BF16),
            pltpu.VMEM((M, D), F32),
            pltpu.VMEM((2, M, D), BF16),
            pltpu.VMEM((2 * FG, M, DH), BF16),
            pltpu.SemaphoreType.DMA((3, 4)),
            pltpu.SemaphoreType.DMA((2, 4)),
            pltpu.SemaphoreType.DMA((XC,)),
            pltpu.SemaphoreType.DMA((FG // 2,)),
            pltpu.SemaphoreType.DMA((1,)),
            pltpu.SemaphoreType.DMA((1 + len(LCH),)),
        ],
        compiler_params=pltpu.CompilerParams(
            vmem_limit_bytes=100 * 1024 * 1024,
            disable_bounds_checks=True,
            disable_semaphore_checks=True,
        ),
        name="mha2",
    )(A_x.reshape(M, D), A_k_cache, A_v_cache, A_wq, A_wo,
      B_x.reshape(M, D), B_k_cache, B_v_cache, B_wq, B_wo)
    return out.reshape(B, SQ, 2 * D)
```

```python
import jax
import jax.numpy as jnp
from jax import lax
import jax.experimental.pallas as pl
import jax.experimental.pallas.tpu as pltpu

B, SQ, D, H, SK, DH = 16, 80, 512, 32, 80, 128
M = B * SQ
C = (DH ** -0.5) * 1.4426950408889634
BF16 = jnp.bfloat16
F32 = jnp.float32

HG = 6
CB = 8
FG = 4
NA = (H - 2 * FG) // HG
NB = (H - 1) // HG
L = H - NB * HG
NJ = NA + NB
XC = 4
XR = M // XC
LCH = (4, 4, 4, 2, 2)
assert 2 * FG + NA * HG == H and NB * HG + L == H and L <= HG and sum(LCH) == B

LAG = dict(Q=1, K=0, S=0, V=-1, O=-2)
MAIN_ORDER = "VKOQS"
EDGE_ORDER = "QKVOS"


def _kernel(xa, ka, va, wqa, woa, xb, kb, vb, wqb, wob, out_hbm,
            x_buf, k_buf, v_buf, wq_buf, wo_buf, acc_ref, out_buf, q_buf,
            sem_w, sem_f, sem_x, sem_p, sem_xb, sem_o):
    one = pl.program_id(0) + 1
    refs_a = (ka, va, wqa, woa)
    refs_b = (kb, vb, wqb, wob)

    def mo(v, m):
        return v if isinstance(v, int) else pl.multiple_of(v, m)

    def once(fn):
        def body(_, c):
            fn()
            return c
        lax.fori_loop(0, one, body, 0)

    def copies(refs, h0, nh, sl, sems):
        k_, v_, wq_, wo_ = refs
        so, w = mo(h0 * DH, DH), nh * DH
        return [
            pltpu.make_async_copy(wq_.at[:, pl.ds(so, w)], wq_buf.at[sl, :, pl.ds(0, w)], sems[0]),
            pltpu.make_async_copy(k_.at[:, pl.ds(h0, nh)], k_buf.at[sl, :, pl.ds(0, nh)], sems[1]),
            pltpu.make_async_copy(v_.at[:, pl.ds(h0, nh)], v_buf.at[sl, :, pl.ds(0, nh)], sems[2]),
            pltpu.make_async_copy(wo_.at[pl.ds(so, w), :], wo_buf.at[sl, pl.ds(0, w), :], sems[3]),
        ]

    def wsems(sl):
        return [sem_w.at[sl, i] for i in range(4)]

    def kvo_copies(g):
        return copies(refs_a, g * FG, FG, g, [sem_f.at[g, i] for i in range(4)])[1:]

    def wq1_copy():
        return copies(refs_a, FG, FG, 1, [sem_f.at[1, i] for i in range(4)])[0]

    def wq_pair(i):
        cols = pl.ds(mo(i * 2 * DH, 2 * DH), 2 * DH)
        return pltpu.make_async_copy(wqa.at[:, cols], wq_buf.at[0, :, cols], sem_p.at[i])

    def x_copy(i):
        r = pl.ds(mo(i * XR, XR), XR)
        return pltpu.make_async_copy(xa.at[r], x_buf.at[0, r], sem_x.at[i])

    xb_cp = pltpu.make_async_copy(xb, x_buf.at[1], sem_xb.at[0])

    def start_group(j, sl):
        @pl.when(j < NA)
        def _():
            for cp in copies(refs_a, 2 * FG + j * HG, HG, sl, wsems(sl)):
                cp.start()

        @pl.when(jnp.logical_and(j >= NA, j < NJ))
        def _():
            for cp in copies(refs_b, (j - NA) * HG, HG, sl, wsems(sl)):
                cp.start()

        @pl.when(j == NJ)
        def _():
            for cp in copies(refs_b, NB * HG, L, sl, wsems(sl)):
                cp.start()

    def wait_group(sl, nh):
        for cp in copies(refs_a, 0, nh, sl, wsems(sl)):
            cp.wait()

    def compute(order, sl, br, first, slots, write_out, q0=None, after_out=None):
        n = len(slots)
        hmin = min(s[0] for s in slots)
        hmax = max(s[0] for s in slots)
        q, sc, p, l, o = {}, {}, {}, {}, {}

        def rows(t):
            _, b0, nb = slots[t]
            return slice(b0 * SQ, (b0 + nb) * SQ)

        def qproj(t):
            hi = slots[t][0]
            if q0 is not None:
                q[t] = q_buf[q0 + hi, rows(t), :]
            else:
                q[t] = jnp.dot(x_buf[br, rows(t), :], wq_buf[sl, :, hi * DH:(hi + 1) * DH],
                               preferred_element_type=F32).astype(BF16)

        def qk(t):
            hi, b0, nb = slots[t]
            qt = q.pop(t)
            sc[t] = [lax.dot_general(qt[j * SQ:(j + 1) * SQ], k_buf[sl, b0 + j, hi],
                                     (((1,), (1,)), ((), ())), preferred_element_type=F32)
                     for j in range(nb)]

        def softmax(t):
            p[t], l[t] = [], []
            for sj in sc.pop(t):
                m = jnp.max(sj, axis=-1, keepdims=True)
                pj = jnp.exp2((sj - m) * C)
                l[t].append(jnp.sum(pj, axis=-1, keepdims=True))
                p[t].append(pj.astype(BF16))

        def pv(t):
            hi, b0, nb = slots[t]
            pt, lt = p.pop(t), l.pop(t)
            outs = []
            for j in range(nb):
                oj = jnp.dot(pt[j], v_buf[sl, b0 + j, hi], preferred_element_type=F32)
                r0 = pl.reciprocal(lt[j], approx=True)
                r1 = r0 * (2.0 - lt[j] * r0)
                outs.append((oj * r1).astype(BF16))
            o[t] = jnp.concatenate(outs, axis=0)

        def oproj(t):
            hi = slots[t][0]
            old = acc_ref[rows(t), :]
            if hi == hmin and first is not None:
                old = jnp.where(first, 0.0, old)
            new = old + jnp.dot(o.pop(t), wo_buf[sl, hi * DH:(hi + 1) * DH, :],
                                preferred_element_type=F32)
            if write_out and hi == hmax:
                out_buf[br, rows(t), :] = new.astype(BF16)
                if after_out is not None:
                    after_out(t)
            if not (write_out == "only" and hi == hmax):
                acc_ref[rows(t), :] = new

        fns = dict(Q=qproj, K=qk, S=softmax, V=pv, O=oproj)
        for t in range(-max(LAG.values()), n - min(LAG.values())):
            for st in order:
                if 0 <= t + LAG[st] < n:
                    fns[st](t + LAG[st])

    def head_major(nh):
        return [(hi, c * CB, CB) for hi in range(nh) for c in range(B // CB)]

    def qdot(xr, g, cols):
        return jnp.dot(xr, wq_buf[g, :, cols], preferred_element_type=F32).astype(BF16)

    def head_cols(h):
        return pl.ds(mo(h * DH, DH), DH)

    def first_phase():
        wq_pair(0).start()
        once(lambda: x_copy(0).start())
        once(lambda: wq_pair(1).start())

        def start_x(i, c):
            x_copy(i).start()
            return c
        lax.fori_loop(1, XC, start_x, 0)
        once(lambda: wq1_copy().start())

        def start_kvo(g, c):
            for cp in kvo_copies(g):
                cp.start()
            return c
        lax.fori_loop(0, 2, start_kvo, 0)
        once(lambda: start_group(one - 1, 2))

        x_copy(0).wait()

        def q_pair(i, c):
            wq_pair(i).wait()
            xr = x_buf[0, 0:XR, :]
            for hh in range(2):
                q_buf[2 * i + hh, 0:XR, :] = qdot(xr, 0, head_cols(2 * i + hh))
            return c
        lax.fori_loop(0, FG // 2, q_pair, 0)
        x_copy(1).wait()
        x_copy(2).wait()

        def q_mid():
            xr = x_buf[0, XR:3 * XR, :]
            for h in range(FG):
                q_buf[h, XR:3 * XR, :] = qdot(xr, 0, head_cols(h))
        once(q_mid)
        x_copy(3).wait()
        wq1_copy().wait()
        xr = x_buf[0, 3 * XR:M, :]
        for h in range(FG):
            q_buf[h, 3 * XR:M, :] = qdot(xr, 0, head_cols(h))
        xr = x_buf[0]
        for h in range(FG):
            q_buf[FG + h] = qdot(xr, 1, head_cols(h))

        def first_attn(g, c):
            for cp in kvo_copies(g):
                cp.wait()
            compute(EDGE_ORDER, g, 0, g == 0, head_major(FG), False, q0=g * FG)
            start_group(g + 1, g)
            return c
        lax.fori_loop(0, 2, first_attn, 0)

    def main_step(j, sl):
        br = (j >= NA).astype(jnp.int32)

        @pl.when(j == NA)
        def _():
            xb_cp.wait()
        wait_group(sl, HG)
        compute(MAIN_ORDER, sl, br, j == NA, head_major(HG), True)
        start_group(j + 3, sl)

        @pl.when(j == 0)
        def _():
            xb_cp.start()

        @pl.when(j == NA - 1)
        def _():
            pltpu.make_async_copy(out_buf.at[0], out_hbm.at[:, pl.ds(0, D)], sem_o.at[0]).start()

    def last_phase():
        lsl = (NJ + 2) % 3
        wait_group(lsl, L)
        slots, b0 = [], 0
        for nb in LCH:
            slots += [(hi, b0, nb) for hi in range(L)]
            b0 += nb

        def out_part(t):
            _, b0, nb = slots[t]
            r = pl.ds(b0 * SQ, nb * SQ)
            return pltpu.make_async_copy(out_buf.at[1, r], out_hbm.at[r, pl.ds(D, D)],
                                         sem_o.at[1 + t // L])

        compute(EDGE_ORDER, lsl, 1, None, slots, "only", after_out=lambda t: out_part(t).start())
        pltpu.make_async_copy(out_buf.at[0], out_hbm.at[:, pl.ds(0, D)], sem_o.at[0]).wait()
        for t in range(L - 1, len(slots), L):
            out_part(t).wait()

    def main_phase():
        def body(j, sl):
            main_step(j, sl)
            return jnp.where(sl == 2, 0, sl + 1)
        lax.fori_loop(0, NJ, body, 2 * one)

    def phase(s, c):
        pl.when(s == 1)(main_phase)
        pl.when(s == 2)(last_phase)
        pl.when(s == 0)(first_phase)
        return c
    lax.fori_loop(0, 3, phase, 0)


@jax.jit
def pallas_concat_heads__mha_block_cached__mha_block_cached__near_ridge_kernel(
    A_x: jax.Array,
    A_k_cache: jax.Array,
    A_v_cache: jax.Array,
    A_wq: jax.Array,
    A_wo: jax.Array,
    B_x: jax.Array,
    B_k_cache: jax.Array,
    B_v_cache: jax.Array,
    B_wq: jax.Array,
    B_wo: jax.Array,
):
    any_spec = pl.BlockSpec(memory_space=pl.ANY)
    out = pl.pallas_call(
        _kernel,
        grid=(1,),
        in_specs=[any_spec] * 10,
        out_specs=any_spec,
        out_shape=jax.ShapeDtypeStruct((M, 2 * D), BF16),
        scratch_shapes=[
            pltpu.VMEM((2, M, D), BF16),
            pltpu.VMEM((3, B, HG, SK, DH), BF16),
            pltpu.VMEM((3, B, HG, SK, DH), BF16),
            pltpu.VMEM((3, D, HG * DH), BF16),
            pltpu.VMEM((3, HG * DH, D), BF16),
            pltpu.VMEM((M, D), F32),
            pltpu.VMEM((2, M, D), BF16),
            pltpu.VMEM((2 * FG, M, DH), BF16),
            pltpu.SemaphoreType.DMA((3, 4)),
            pltpu.SemaphoreType.DMA((2, 4)),
            pltpu.SemaphoreType.DMA((XC,)),
            pltpu.SemaphoreType.DMA((FG // 2,)),
            pltpu.SemaphoreType.DMA((1,)),
            pltpu.SemaphoreType.DMA((1 + len(LCH),)),
        ],
        compiler_params=pltpu.CompilerParams(
            vmem_limit_bytes=100 * 1024 * 1024,
            disable_bounds_checks=True,
            disable_semaphore_checks=True,
        ),
        name="mha2",
    )(A_x.reshape(M, D), A_k_cache, A_v_cache, A_wq, A_wo,
      B_x.reshape(M, D), B_k_cache, B_v_cache, B_wq, B_wo)
    return out.reshape(B, SQ, 2 * D)
```

```python
import jax
import jax.numpy as jnp
from jax import lax
import jax.experimental.pallas as pl
import jax.experimental.pallas.tpu as pltpu

B, SQ, D, H, SK, DH = 16, 80, 512, 32, 80, 128
M = B * SQ
C = (DH ** -0.5) * 1.4426950408889634
BF16 = jnp.bfloat16
F32 = jnp.float32

HG = 6
CB = 8
FG = 4
NA = (H - 2 * FG) // HG
NB = (H - 1) // HG
L = H - NB * HG
NJ = NA + NB
XC = 4
XR = M // XC
LCH = (4, 4, 4, 2, 2)
assert 2 * FG + NA * HG == H and NB * HG + L == H and L <= HG and sum(LCH) == B

LAG = dict(Q=1, K=0, S=0, V=-1, O=-2)
MAIN_ORDER = "VKOQS"
EDGE_ORDER = "QKVOS"


def _kernel(xa, ka, va, wqa, woa, xb, kb, vb, wqb, wob, out_hbm,
            x_buf, k_buf, v_buf, wq_buf, wo_buf, acc_ref, out_buf, q_buf,
            sem_w, sem_f, sem_x, sem_p, sem_xb, sem_o):
    one = pl.program_id(0) + 1
    refs_a = (ka, va, wqa, woa)
    refs_b = (kb, vb, wqb, wob)

    def mo(v, m):
        return v if isinstance(v, int) else pl.multiple_of(v, m)

    def once(fn):
        def body(_, c):
            fn()
            return c
        lax.fori_loop(0, one, body, 0)

    def copy(kind, refs, h0, nh, sl, sem):
        k_, v_, wq_, wo_ = refs
        so, w = mo(h0 * DH, DH), nh * DH
        if kind == 0:
            return pltpu.make_async_copy(wq_.at[:, pl.ds(so, w)], wq_buf.at[sl, :, pl.ds(0, w)], sem)
        if kind == 1:
            return pltpu.make_async_copy(k_.at[:, pl.ds(h0, nh)], k_buf.at[sl, :, pl.ds(0, nh)], sem)
        if kind == 2:
            return pltpu.make_async_copy(v_.at[:, pl.ds(h0, nh)], v_buf.at[sl, :, pl.ds(0, nh)], sem)
        return pltpu.make_async_copy(wo_.at[pl.ds(so, w), :], wo_buf.at[sl, pl.ds(0, w), :], sem)

    def group_copies(refs, h0, nh, sl):
        return [copy(kind, refs, h0, nh, sl, sem_w.at[sl, kind]) for kind in range(4)]

    def kvo_copies(g):
        return [copy(kind, refs_a, g * FG, FG, g, sem_f.at[g, kind - 1]) for kind in range(1, 4)]

    def wq1_copy():
        return copy(0, refs_a, FG, FG, 1, sem_p.at[FG // 2])

    def wq_pair(i):
        cols = pl.ds(mo(i * 2 * DH, 2 * DH), 2 * DH)
        return pltpu.make_async_copy(wqa.at[:, cols], wq_buf.at[0, :, cols], sem_p.at[i])

    def x_copy(i):
        r = pl.ds(mo(i * XR, XR), XR)
        return pltpu.make_async_copy(xa.at[r], x_buf.at[0, r], sem_x.at[i])

    xb_cp = pltpu.make_async_copy(xb, x_buf.at[1], sem_xb.at[0])

    def start_group(j, sl):
        @pl.when(j < NA)
        def _():
            for cp in group_copies(refs_a, 2 * FG + j * HG, HG, sl):
                cp.start()

        @pl.when(jnp.logical_and(j >= NA, j < NJ))
        def _():
            for cp in group_copies(refs_b, (j - NA) * HG, HG, sl):
                cp.start()

        @pl.when(j == NJ)
        def _():
            for cp in group_copies(refs_b, NB * HG, L, sl):
                cp.start()

    def wait_group(sl, nh):
        for cp in group_copies(refs_a, 0, nh, sl):
            cp.wait()

    def compute(order, sl, br, first, slots, write_out, q0=None, after_out=None):
        n = len(slots)
        hmin = min(s[0] for s in slots)
        hmax = max(s[0] for s in slots)
        q, sc, p, l, o = {}, {}, {}, {}, {}

        def rows(t):
            _, b0, nb = slots[t]
            return slice(b0 * SQ, (b0 + nb) * SQ)

        def qproj(t):
            hi = slots[t][0]
            if q0 is not None:
                q[t] = q_buf[q0 + hi, rows(t), :]
            else:
                q[t] = jnp.dot(x_buf[br, rows(t), :], wq_buf[sl, :, hi * DH:(hi + 1) * DH],
                               preferred_element_type=F32).astype(BF16)

        def qk(t):
            hi, b0, nb = slots[t]
            qt = q.pop(t)
            sc[t] = [lax.dot_general(qt[j * SQ:(j + 1) * SQ], k_buf[sl, b0 + j, hi],
                                     (((1,), (1,)), ((), ())), preferred_element_type=F32)
                     for j in range(nb)]

        def softmax(t):
            p[t], l[t] = [], []
            for sj in sc.pop(t):
                m = jnp.max(sj, axis=-1, keepdims=True)
                pj = jnp.exp2((sj - m) * C)
                l[t].append(jnp.sum(pj, axis=-1, keepdims=True))
                p[t].append(pj.astype(BF16))

        def pv(t):
            hi, b0, nb = slots[t]
            pt, lt = p.pop(t), l.pop(t)
            outs = []
            for j in range(nb):
                oj = jnp.dot(pt[j], v_buf[sl, b0 + j, hi], preferred_element_type=F32)
                r0 = pl.reciprocal(lt[j], approx=True)
                r1 = r0 * (2.0 - lt[j] * r0)
                outs.append((oj * r1).astype(BF16))
            o[t] = jnp.concatenate(outs, axis=0)

        def oproj(t):
            hi = slots[t][0]
            old = acc_ref[rows(t), :]
            if hi == hmin and first is not None:
                old = jnp.where(first, 0.0, old)
            new = old + jnp.dot(o.pop(t), wo_buf[sl, hi * DH:(hi + 1) * DH, :],
                                preferred_element_type=F32)
            if write_out and hi == hmax:
                out_buf[br, rows(t), :] = new.astype(BF16)
                if after_out is not None:
                    after_out(t)
            if not (write_out == "only" and hi == hmax):
                acc_ref[rows(t), :] = new

        fns = dict(Q=qproj, K=qk, S=softmax, V=pv, O=oproj)
        for t in range(-max(LAG.values()), n - min(LAG.values())):
            for st in order:
                if 0 <= t + LAG[st] < n:
                    fns[st](t + LAG[st])

    def head_major(nh):
        return [(hi, c * CB, CB) for hi in range(nh) for c in range(B // CB)]

    def qdot(xr, g, cols):
        return jnp.dot(xr, wq_buf[g, :, cols], preferred_element_type=F32).astype(BF16)

    def head_cols(h):
        return pl.ds(mo(h * DH, DH), DH)

    def first_phase():
        wq_pair(0).start()
        once(lambda: x_copy(0).start())
        once(lambda: wq_pair(1).start())

        def start_x(i, c):
            x_copy(i).start()
            return c
        lax.fori_loop(1, XC, start_x, 0)
        once(lambda: wq1_copy().start())

        def start_kvo(g, c):
            for cp in kvo_copies(g):
                cp.start()
            return c
        lax.fori_loop(0, 2, start_kvo, 0)
        once(lambda: start_group(one - 1, 2))

        x_copy(0).wait()

        def q_pair(i, c):
            wq_pair(i).wait()
            xr = x_buf[0, 0:XR, :]
            for hh in range(2):
                q_buf[2 * i + hh, 0:XR, :] = qdot(xr, 0, head_cols(2 * i + hh))
            return c
        lax.fori_loop(0, FG // 2, q_pair, 0)
        x_copy(1).wait()
        x_copy(2).wait()

        def q_mid():
            xr = x_buf[0, XR:3 * XR, :]
            for h in range(FG):
                q_buf[h, XR:3 * XR, :] = qdot(xr, 0, head_cols(h))
        once(q_mid)
        x_copy(3).wait()
        wq1_copy().wait()
        xr = x_buf[0, 3 * XR:M, :]
        for h in range(FG):
            q_buf[h, 3 * XR:M, :] = qdot(xr, 0, head_cols(h))
        xr = x_buf[0]
        for h in range(FG):
            q_buf[FG + h] = qdot(xr, 1, head_cols(h))

        def first_attn(g, c):
            for cp in kvo_copies(g):
                cp.wait()
            compute(EDGE_ORDER, g, 0, g == 0, head_major(FG), False, q0=g * FG)
            start_group(g + 1, g)
            return c
        lax.fori_loop(0, 2, first_attn, 0)

    def main_step(j, sl):
        br = (j >= NA).astype(jnp.int32)

        @pl.when(j == NA)
        def _():
            xb_cp.wait()
        wait_group(sl, HG)
        compute(MAIN_ORDER, sl, br, j == NA, head_major(HG), True)
        start_group(j + 3, sl)

        @pl.when(j == 0)
        def _():
            xb_cp.start()

        @pl.when(j == NA - 1)
        def _():
            pltpu.make_async_copy(out_buf.at[0], out_hbm.at[:, pl.ds(0, D)], sem_o.at[0]).start()

    def last_phase():
        lsl = (NJ + 2) % 3
        wait_group(lsl, L)
        slots, b0 = [], 0
        for nb in LCH:
            slots += [(hi, b0, nb) for hi in range(L)]
            b0 += nb

        def out_part(t):
            _, b0, nb = slots[t]
            r = pl.ds(b0 * SQ, nb * SQ)
            return pltpu.make_async_copy(out_buf.at[1, r], out_hbm.at[r, pl.ds(D, D)],
                                         sem_o.at[1 + t // L])

        compute(EDGE_ORDER, lsl, 1, None, slots, "only", after_out=lambda t: out_part(t).start())
        pltpu.make_async_copy(out_buf.at[0], out_hbm.at[:, pl.ds(0, D)], sem_o.at[0]).wait()
        for t in range(L - 1, len(slots), L):
            out_part(t).wait()

    def main_phase():
        def body(j, sl):
            main_step(j, sl)
            return jnp.where(sl == 2, 0, sl + 1)
        lax.fori_loop(0, NJ, body, 2 * one)

    def phase(s, c):
        pl.when(s == 1)(main_phase)
        pl.when(s == 2)(last_phase)
        pl.when(s == 0)(first_phase)
        return c
    lax.fori_loop(0, 3, phase, 0)


@jax.jit
def pallas_concat_heads__mha_block_cached__mha_block_cached__near_ridge_kernel(
    A_x: jax.Array,
    A_k_cache: jax.Array,
    A_v_cache: jax.Array,
    A_wq: jax.Array,
    A_wo: jax.Array,
    B_x: jax.Array,
    B_k_cache: jax.Array,
    B_v_cache: jax.Array,
    B_wq: jax.Array,
    B_wo: jax.Array,
):
    any_spec = pl.BlockSpec(memory_space=pl.ANY)
    out = pl.pallas_call(
        _kernel,
        grid=(1,),
        in_specs=[any_spec] * 10,
        out_specs=any_spec,
        out_shape=jax.ShapeDtypeStruct((M, 2 * D), BF16),
        scratch_shapes=[
            pltpu.VMEM((2, M, D), BF16),
            pltpu.VMEM((3, B, HG, SK, DH), BF16),
            pltpu.VMEM((3, B, HG, SK, DH), BF16),
            pltpu.VMEM((3, D, HG * DH), BF16),
            pltpu.VMEM((3, HG * DH, D), BF16),
            pltpu.VMEM((M, D), F32),
            pltpu.VMEM((2, M, D), BF16),
            pltpu.VMEM((2 * FG, M, DH), BF16),
            pltpu.SemaphoreType.DMA((3, 4)),
            pltpu.SemaphoreType.DMA((2, 3)),
            pltpu.SemaphoreType.DMA((XC,)),
            pltpu.SemaphoreType.DMA((FG // 2 + 1,)),
            pltpu.SemaphoreType.DMA((1,)),
            pltpu.SemaphoreType.DMA((1 + len(LCH),)),
        ],
        compiler_params=pltpu.CompilerParams(
            vmem_limit_bytes=100 * 1024 * 1024,
            disable_bounds_checks=True,
            disable_semaphore_checks=True,
        ),
        name="mha2",
    )(A_x.reshape(M, D), A_k_cache, A_v_cache, A_wq, A_wo,
      B_x.reshape(M, D), B_k_cache, B_v_cache, B_wq, B_wo)
    return out.reshape(B, SQ, 2 * D)
```

```python
import jax
import jax.numpy as jnp
from jax import lax
import jax.experimental.pallas as pl
import jax.experimental.pallas.tpu as pltpu

B, SQ, D, H, SK, DH = 16, 80, 512, 32, 80, 128
M = B * SQ
C = (DH ** -0.5) * 1.4426950408889634
BF16 = jnp.bfloat16
F32 = jnp.float32

HG = 7
CB = 8
FG = (4, 7)
NA = (H - sum(FG)) // HG
NB = (H - 1) // HG
L = H - NB * HG
NJ = NA + NB
XC = 4
XR = M // XC
LCH = (8, 4, 3, 1)
assert sum(FG) + NA * HG == H and NB * HG + L == H and max(FG + (L,)) <= HG
assert sum(LCH) == B and FG[0] % 2 == 0

LAG = dict(Q=1, K=0, S=0, V=-1, O=-2)
MAIN_ORDER = "VKOQS"
EDGE_ORDER = "QKVOS"


def _kernel(xa, ka, va, wqa, woa, xb, kb, vb, wqb, wob, out_hbm,
            x_buf, k_buf, v_buf, wq_buf, wo_buf, acc_ref, out_buf, q_buf,
            sem_w, sem_f, sem_x, sem_p, sem_xb, sem_o):
    one = pl.program_id(0) + 1
    refs_a = (ka, va, wqa, woa)
    refs_b = (kb, vb, wqb, wob)

    def mo(v, m):
        return v if isinstance(v, int) else pl.multiple_of(v, m)

    def once(fn):
        def body(_, c):
            fn()
            return c
        lax.fori_loop(0, one, body, 0)

    def copy(kind, refs, h0, nh, sl, sem):
        k_, v_, wq_, wo_ = refs
        so, w = mo(h0 * DH, DH), nh * DH
        if kind == 0:
            return pltpu.make_async_copy(wq_.at[:, pl.ds(so, w)], wq_buf.at[sl, :, pl.ds(0, w)], sem)
        if kind == 1:
            return pltpu.make_async_copy(k_.at[:, pl.ds(h0, nh)], k_buf.at[sl, :, pl.ds(0, nh)], sem)
        if kind == 2:
            return pltpu.make_async_copy(v_.at[:, pl.ds(h0, nh)], v_buf.at[sl, :, pl.ds(0, nh)], sem)
        return pltpu.make_async_copy(wo_.at[pl.ds(so, w), :], wo_buf.at[sl, pl.ds(0, w), :], sem)

    def group_copies(refs, h0, nh, sl):
        return [copy(kind, refs, h0, nh, sl, sem_w.at[sl, kind]) for kind in range(4)]

    def kvo_copies(g):
        return [copy(kind, refs_a, g * FG[0], FG[g], g, sem_f.at[g, kind - 1]) for kind in range(1, 4)]

    def wq1_copy():
        return copy(0, refs_a, FG[0], FG[1], 1, sem_p.at[FG[0] // 2])

    def wq_pair(i):
        cols = pl.ds(mo(i * 2 * DH, 2 * DH), 2 * DH)
        return pltpu.make_async_copy(wqa.at[:, cols], wq_buf.at[0, :, cols], sem_p.at[i])

    def x_copy(i):
        r = pl.ds(mo(i * XR, XR), XR)
        return pltpu.make_async_copy(xa.at[r], x_buf.at[0, r], sem_x.at[i])

    xb_cp = pltpu.make_async_copy(xb, x_buf.at[1], sem_xb.at[0])

    def start_group(j, sl):
        @pl.when(j < NA)
        def _():
            for cp in group_copies(refs_a, sum(FG) + j * HG, HG, sl):
                cp.start()

        @pl.when(jnp.logical_and(j >= NA, j < NJ))
        def _():
            for cp in group_copies(refs_b, (j - NA) * HG, HG, sl):
                cp.start()

        @pl.when(j == NJ)
        def _():
            for cp in group_copies(refs_b, NB * HG, L, sl):
                cp.start()

    def wait_group(sl, nh):
        for cp in group_copies(refs_a, 0, nh, sl):
            cp.wait()

    def compute(order, sl, br, first, slots, write_out, q0=None, after_out=None):
        n = len(slots)
        hmin = min(s[0] for s in slots)
        hmax = max(s[0] for s in slots)
        q, sc, p, l, o = {}, {}, {}, {}, {}

        def rows(t):
            _, b0, nb = slots[t]
            return slice(b0 * SQ, (b0 + nb) * SQ)

        def qproj(t):
            hi = slots[t][0]
            if q0 is not None:
                q[t] = q_buf[q0 + hi, rows(t), :]
            else:
                q[t] = jnp.dot(x_buf[br, rows(t), :], wq_buf[sl, :, hi * DH:(hi + 1) * DH],
                               preferred_element_type=F32).astype(BF16)

        def qk(t):
            hi, b0, nb = slots[t]
            qt = q.pop(t)
            sc[t] = [lax.dot_general(qt[j * SQ:(j + 1) * SQ], k_buf[sl, b0 + j, hi],
                                     (((1,), (1,)), ((), ())), preferred_element_type=F32)
                     for j in range(nb)]

        def softmax(t):
            p[t], l[t] = [], []
            for sj in sc.pop(t):
                m = jnp.max(sj, axis=-1, keepdims=True)
                pj = jnp.exp2((sj - m) * C)
                l[t].append(jnp.sum(pj, axis=-1, keepdims=True))
                p[t].append(pj.astype(BF16))

        def pv(t):
            hi, b0, nb = slots[t]
            pt, lt = p.pop(t), l.pop(t)
            outs = []
            for j in range(nb):
                oj = jnp.dot(pt[j], v_buf[sl, b0 + j, hi], preferred_element_type=F32)
                r0 = pl.reciprocal(lt[j], approx=True)
                r1 = r0 * (2.0 - lt[j] * r0)
                outs.append((oj * r1).astype(BF16))
            o[t] = jnp.concatenate(outs, axis=0) if nb > 1 else outs[0]

        def oproj(t):
            hi = slots[t][0]
            old = acc_ref[rows(t), :]
            if hi == hmin and first is not None:
                old = jnp.where(first, 0.0, old)
            new = old + jnp.dot(o.pop(t), wo_buf[sl, hi * DH:(hi + 1) * DH, :],
                                preferred_element_type=F32)
            if write_out and hi == hmax:
                out_buf[br, rows(t), :] = new.astype(BF16)
                if after_out is not None:
                    after_out(t)
            if not (write_out == "only" and hi == hmax):
                acc_ref[rows(t), :] = new

        fns = dict(Q=qproj, K=qk, S=softmax, V=pv, O=oproj)
        for t in range(-max(LAG.values()), n - min(LAG.values())):
            for st in order:
                if 0 <= t + LAG[st] < n:
                    fns[st](t + LAG[st])

    def head_major(nh):
        return [(hi, c * CB, CB) for hi in range(nh) for c in range(B // CB)]

    def qdot(xr, g, cols):
        return jnp.dot(xr, wq_buf[g, :, cols], preferred_element_type=F32).astype(BF16)

    def head_cols(h):
        return pl.ds(mo(h * DH, DH), DH)

    def first_phase():
        wq_pair(0).start()
        once(lambda: x_copy(0).start())

        def start_wq(i, c):
            wq_pair(i).start()
            return c
        lax.fori_loop(1, FG[0] // 2, start_wq, 0)

        def start_x(i, c):
            x_copy(i).start()
            return c
        lax.fori_loop(1, XC, start_x, 0)
        once(lambda: wq1_copy().start())
        for g in range(2):
            once(lambda g=g: [cp.start() for cp in kvo_copies(g)])
        once(lambda: start_group(one - 1, 2))

        x_copy(0).wait()

        def q_pair(i, c):
            wq_pair(i).wait()
            xr = x_buf[0, 0:XR, :]
            for hh in range(2):
                q_buf[2 * i + hh, 0:XR, :] = qdot(xr, 0, head_cols(2 * i + hh))
            return c
        lax.fori_loop(0, FG[0] // 2, q_pair, 0)
        x_copy(1).wait()
        x_copy(2).wait()

        def q_mid():
            xr = x_buf[0, XR:3 * XR, :]
            for h in range(FG[0]):
                q_buf[h, XR:3 * XR, :] = qdot(xr, 0, head_cols(h))
        once(q_mid)
        x_copy(3).wait()
        wq1_copy().wait()
        xr = x_buf[0, 3 * XR:M, :]
        for h in range(FG[0]):
            q_buf[h, 3 * XR:M, :] = qdot(xr, 0, head_cols(h))
        xr = x_buf[0]
        for h in range(FG[1]):
            q_buf[FG[0] + h] = qdot(xr, 1, head_cols(h))

        for g in range(2):
            def first_attn(g=g):
                for cp in kvo_copies(g):
                    cp.wait()
                compute(EDGE_ORDER, g, 0, (one == 1) if g == 0 else None, head_major(FG[g]),
                        False, q0=g * FG[0])
                start_group(one + g, g)
            once(first_attn)

    def main_step(j, sl):
        br = (j >= NA).astype(jnp.int32)

        @pl.when(j == NA)
        def _():
            xb_cp.wait()
        wait_group(sl, HG)
        compute(MAIN_ORDER, sl, br, j == NA, head_major(HG), True)
        start_group(j + 3, sl)

        @pl.when(j == 0)
        def _():
            xb_cp.start()

        @pl.when(j == NA - 1)
        def _():
            pltpu.make_async_copy(out_buf.at[0], out_hbm.at[:, pl.ds(0, D)], sem_o.at[0]).start()

    def main_phase():
        def body(j, sl):
            main_step(j, sl)
            return jnp.where(sl == 2, 0, sl + 1)
        lax.fori_loop(0, NJ, body, 2 * one)

    def last_phase():
        lsl = (NJ + 2) % 3
        wait_group(lsl, L)
        slots, b0 = [], 0
        for nb in LCH:
            slots += [(hi, b0, nb) for hi in range(L)]
            b0 += nb

        def out_part(t):
            _, b0, nb = slots[t]
            r = pl.ds(b0 * SQ, nb * SQ)
            return pltpu.make_async_copy(out_buf.at[1, r], out_hbm.at[r, pl.ds(D, D)],
                                         sem_o.at[1 + t // L])

        compute(EDGE_ORDER, lsl, 1, None, slots, "only", after_out=lambda t: out_part(t).start())
        pltpu.make_async_copy(out_buf.at[0], out_hbm.at[:, pl.ds(0, D)], sem_o.at[0]).wait()
        for t in range(L - 1, len(slots), L):
            out_part(t).wait()

    def phase(s, c):
        pl.when(s == 1)(main_phase)
        pl.when(s == 2)(last_phase)
        pl.when(s == 0)(first_phase)
        return c
    lax.fori_loop(0, 3, phase, 0)


@jax.jit
def pallas_concat_heads__mha_block_cached__mha_block_cached__near_ridge_kernel(
    A_x: jax.Array,
    A_k_cache: jax.Array,
    A_v_cache: jax.Array,
    A_wq: jax.Array,
    A_wo: jax.Array,
    B_x: jax.Array,
    B_k_cache: jax.Array,
    B_v_cache: jax.Array,
    B_wq: jax.Array,
    B_wo: jax.Array,
):
    any_spec = pl.BlockSpec(memory_space=pl.ANY)
    out = pl.pallas_call(
        _kernel,
        grid=(1,),
        in_specs=[any_spec] * 10,
        out_specs=any_spec,
        out_shape=jax.ShapeDtypeStruct((M, 2 * D), BF16),
        scratch_shapes=[
            pltpu.VMEM((2, M, D), BF16),
            pltpu.VMEM((3, B, HG, SK, DH), BF16),
            pltpu.VMEM((3, B, HG, SK, DH), BF16),
            pltpu.VMEM((3, D, HG * DH), BF16),
            pltpu.VMEM((3, HG * DH, D), BF16),
            pltpu.VMEM((M, D), F32),
            pltpu.VMEM((2, M, D), BF16),
            pltpu.VMEM((sum(FG), M, DH), BF16),
            pltpu.SemaphoreType.DMA((3, 4)),
            pltpu.SemaphoreType.DMA((2, 3)),
            pltpu.SemaphoreType.DMA((XC,)),
            pltpu.SemaphoreType.DMA((FG[0] // 2 + 1,)),
            pltpu.SemaphoreType.DMA((1,)),
            pltpu.SemaphoreType.DMA((1 + len(LCH),)),
        ],
        compiler_params=pltpu.CompilerParams(
            vmem_limit_bytes=100 * 1024 * 1024,
            disable_bounds_checks=True,
            disable_semaphore_checks=True,
        ),
        name="mha2",
    )(A_x.reshape(M, D), A_k_cache, A_v_cache, A_wq, A_wo,
      B_x.reshape(M, D), B_k_cache, B_v_cache, B_wq, B_wo)
    return out.reshape(B, SQ, 2 * D)
```

```python
import jax
import jax.numpy as jnp
from jax import lax
import jax.experimental.pallas as pl
import jax.experimental.pallas.tpu as pltpu

B, SQ, D, H, SK, DH = 16, 80, 512, 32, 80, 128
M = B * SQ
C = (DH ** -0.5) * 1.4426950408889634
BF16 = jnp.bfloat16
F32 = jnp.float32

HG = 7
CB = 8
FG = (4, 7)
NA = (H - sum(FG)) // HG
NB = (H - 1) // HG
L = H - NB * HG
NJ = NA + NB
XC = 4
XR = M // XC
LCH = (8, 4, 3, 1)
assert sum(FG) + NA * HG == H and NB * HG + L == H and max(FG + (L,)) <= HG
assert sum(LCH) == B and FG[0] % 2 == 0

LAG = dict(Q=1, K=0, S=0, V=-1, O=-2)
MAIN_ORDER = "VKOQS"
EDGE_ORDER = "QKVOS"


def _kernel(xa, ka, va, wqa, woa, xb, kb, vb, wqb, wob, out_hbm,
            x_buf, k_buf, v_buf, wq_buf, wo_buf, acc_ref, out_buf, q_buf,
            sem_w, sem_f, sem_x, sem_p, sem_xb, sem_o):
    one = pl.program_id(0) + 1
    refs_a = (ka, va, wqa, woa)
    refs_b = (kb, vb, wqb, wob)

    def mo(v, m):
        return v if isinstance(v, int) else pl.multiple_of(v, m)

    def once(fn):
        def body(_, c):
            fn()
            return c
        lax.fori_loop(0, one, body, 0)

    def copy(kind, refs, h0, nh, sl, sem):
        k_, v_, wq_, wo_ = refs
        so, w = mo(h0 * DH, DH), nh * DH
        if kind == 0:
            return pltpu.make_async_copy(wq_.at[:, pl.ds(so, w)], wq_buf.at[sl, :, pl.ds(0, w)], sem)
        if kind == 1:
            return pltpu.make_async_copy(k_.at[:, pl.ds(h0, nh)], k_buf.at[sl, :, pl.ds(0, nh)], sem)
        if kind == 2:
            return pltpu.make_async_copy(v_.at[:, pl.ds(h0, nh)], v_buf.at[sl, :, pl.ds(0, nh)], sem)
        return pltpu.make_async_copy(wo_.at[pl.ds(so, w), :], wo_buf.at[sl, pl.ds(0, w), :], sem)

    def group_copies(refs, h0, nh, sl):
        return [copy(kind, refs, h0, nh, sl, sem_w.at[sl, kind]) for kind in range(4)]

    def kvo_copies(g):
        return [copy(kind, refs_a, g * FG[0], FG[g], g, sem_f.at[g, kind - 1]) for kind in range(1, 4)]

    def wq1_copy():
        return copy(0, refs_a, FG[0], FG[1], 1, sem_p.at[FG[0] // 2])

    def wq_pair(i):
        cols = pl.ds(mo(i * 2 * DH, 2 * DH), 2 * DH)
        return pltpu.make_async_copy(wqa.at[:, cols], wq_buf.at[0, :, cols], sem_p.at[i])

    def x_copy(i):
        r = pl.ds(mo(i * XR, XR), XR)
        return pltpu.make_async_copy(xa.at[r], x_buf.at[0, r], sem_x.at[i])

    xb_cp = pltpu.make_async_copy(xb, x_buf.at[1], sem_xb.at[0])

    def start_group(j, sl):
        @pl.when(j < NA)
        def _():
            for cp in group_copies(refs_a, sum(FG) + j * HG, HG, sl):
                cp.start()

        @pl.when(jnp.logical_and(j >= NA, j < NJ))
        def _():
            for cp in group_copies(refs_b, (j - NA) * HG, HG, sl):
                cp.start()

        @pl.when(j == NJ)
        def _():
            for cp in group_copies(refs_b, NB * HG, L, sl):
                cp.start()

    def wait_group(sl, nh):
        for cp in group_copies(refs_a, 0, nh, sl):
            cp.wait()

    def compute(order, sl, br, first, slots, write_out, q0=None, after_out=None):
        n = len(slots)
        hmin = min(s[0] for s in slots)
        hmax = max(s[0] for s in slots)
        q, sc, p, l, o = {}, {}, {}, {}, {}

        def rows(t):
            _, b0, nb = slots[t]
            return slice(b0 * SQ, (b0 + nb) * SQ)

        def qproj(t):
            hi = slots[t][0]
            if q0 is not None:
                q[t] = q_buf[q0 + hi, rows(t), :]
            else:
                q[t] = jnp.dot(x_buf[br, rows(t), :], wq_buf[sl, :, hi * DH:(hi + 1) * DH],
                               preferred_element_type=F32).astype(BF16)

        def qk(t):
            hi, b0, nb = slots[t]
            qt = q.pop(t)
            sc[t] = [lax.dot_general(qt[j * SQ:(j + 1) * SQ], k_buf[sl, b0 + j, hi],
                                     (((1,), (1,)), ((), ())), preferred_element_type=F32)
                     for j in range(nb)]

        def softmax(t):
            p[t], l[t] = [], []
            for sj in sc.pop(t):
                m = jnp.max(sj, axis=-1, keepdims=True)
                pj = jnp.exp2((sj - m) * C)
                l[t].append(jnp.sum(pj, axis=-1, keepdims=True))
                p[t].append(pj.astype(BF16))

        def pv(t):
            hi, b0, nb = slots[t]
            pt, lt = p.pop(t), l.pop(t)
            outs = []
            for j in range(nb):
                oj = jnp.dot(pt[j], v_buf[sl, b0 + j, hi], preferred_element_type=F32)
                r0 = pl.reciprocal(lt[j], approx=True)
                r1 = r0 * (2.0 - lt[j] * r0)
                outs.append((oj * r1).astype(BF16))
            o[t] = jnp.concatenate(outs, axis=0) if nb > 1 else outs[0]

        def oproj(t):
            hi = slots[t][0]
            fresh = hi == hmin and first is True
            if not fresh:
                old = acc_ref[rows(t), :]
                if hi == hmin and first is not None:
                    old = jnp.where(first, 0.0, old)
            new = jnp.dot(o.pop(t), wo_buf[sl, hi * DH:(hi + 1) * DH, :], preferred_element_type=F32)
            if not fresh:
                new = old + new
            if write_out and hi == hmax:
                out_buf[br, rows(t), :] = new.astype(BF16)
                if after_out is not None:
                    after_out(t)
            if not (write_out == "only" and hi == hmax):
                acc_ref[rows(t), :] = new

        fns = dict(Q=qproj, K=qk, S=softmax, V=pv, O=oproj)
        for t in range(-max(LAG.values()), n - min(LAG.values())):
            for st in order:
                if 0 <= t + LAG[st] < n:
                    fns[st](t + LAG[st])

    def head_major(nh):
        return [(hi, c * CB, CB) for hi in range(nh) for c in range(B // CB)]

    def qdot(xr, g, cols):
        return jnp.dot(xr, wq_buf[g, :, cols], preferred_element_type=F32).astype(BF16)

    def head_cols(h):
        return pl.ds(mo(h * DH, DH), DH)

    def first_phase():
        wq_pair(0).start()
        once(lambda: x_copy(0).start())

        def start_wq(i, c):
            wq_pair(i).start()
            return c
        lax.fori_loop(1, FG[0] // 2, start_wq, 0)

        def start_x(i, c):
            x_copy(i).start()
            return c
        lax.fori_loop(1, XC, start_x, 0)
        once(lambda: wq1_copy().start())
        for g in range(2):
            once(lambda g=g: [cp.start() for cp in kvo_copies(g)])
        once(lambda: start_group(one - 1, 2))

        x_copy(0).wait()

        def q_pair(i, c):
            wq_pair(i).wait()
            xr = x_buf[0, 0:XR, :]
            for hh in range(2):
                q_buf[2 * i + hh, 0:XR, :] = qdot(xr, 0, head_cols(2 * i + hh))
            return c
        lax.fori_loop(0, FG[0] // 2, q_pair, 0)
        x_copy(1).wait()
        x_copy(2).wait()

        def q_mid():
            xr = x_buf[0, XR:3 * XR, :]
            for h in range(FG[0]):
                q_buf[h, XR:3 * XR, :] = qdot(xr, 0, head_cols(h))
        once(q_mid)
        x_copy(3).wait()
        wq1_copy().wait()
        xr = x_buf[0, 3 * XR:M, :]
        for h in range(FG[0]):
            q_buf[h, 3 * XR:M, :] = qdot(xr, 0, head_cols(h))
        xr = x_buf[0]
        for h in range(FG[1]):
            q_buf[FG[0] + h] = qdot(xr, 1, head_cols(h))

        for g in range(2):
            def first_attn(g=g):
                for cp in kvo_copies(g):
                    cp.wait()
                compute(EDGE_ORDER, g, 0, True if g == 0 else None, head_major(FG[g]),
                        False, q0=g * FG[0])
                start_group(one + g, g)
            once(first_attn)

    def main_step(j, sl):
        br = (j >= NA).astype(jnp.int32)

        @pl.when(j == NA)
        def _():
            xb_cp.wait()
        wait_group(sl, HG)
        compute(MAIN_ORDER, sl, br, j == NA, head_major(HG), True)
        start_group(j + 3, sl)

        @pl.when(j == 0)
        def _():
            xb_cp.start()

        @pl.when(j == NA - 1)
        def _():
            pltpu.make_async_copy(out_buf.at[0], out_hbm.at[:, pl.ds(0, D)], sem_o.at[0]).start()

    def main_phase():
        def body(j, sl):
            main_step(j, sl)
            return jnp.where(sl == 2, 0, sl + 1)
        lax.fori_loop(0, NJ, body, 2 * one)

    def last_phase():
        lsl = (NJ + 2) % 3
        wait_group(lsl, L)
        slots, b0 = [], 0
        for nb in LCH:
            slots += [(hi, b0, nb) for hi in range(L)]
            b0 += nb

        def out_part(t):
            _, b0, nb = slots[t]
            r = pl.ds(b0 * SQ, nb * SQ)
            return pltpu.make_async_copy(out_buf.at[1, r], out_hbm.at[r, pl.ds(D, D)],
                                         sem_o.at[1 + t // L])

        compute(EDGE_ORDER, lsl, 1, None, slots, "only", after_out=lambda t: out_part(t).start())
        pltpu.make_async_copy(out_buf.at[0], out_hbm.at[:, pl.ds(0, D)], sem_o.at[0]).wait()
        for t in range(L - 1, len(slots), L):
            out_part(t).wait()

    def phase(s, c):
        pl.when(s == 1)(main_phase)
        pl.when(s == 2)(last_phase)
        pl.when(s == 0)(first_phase)
        return c
    lax.fori_loop(0, 3, phase, 0)


@jax.jit
def pallas_concat_heads__mha_block_cached__mha_block_cached__near_ridge_kernel(
    A_x: jax.Array,
    A_k_cache: jax.Array,
    A_v_cache: jax.Array,
    A_wq: jax.Array,
    A_wo: jax.Array,
    B_x: jax.Array,
    B_k_cache: jax.Array,
    B_v_cache: jax.Array,
    B_wq: jax.Array,
    B_wo: jax.Array,
):
    any_spec = pl.BlockSpec(memory_space=pl.ANY)
    out = pl.pallas_call(
        _kernel,
        grid=(1,),
        in_specs=[any_spec] * 10,
        out_specs=any_spec,
        out_shape=jax.ShapeDtypeStruct((M, 2 * D), BF16),
        scratch_shapes=[
            pltpu.VMEM((2, M, D), BF16),
            pltpu.VMEM((3, B, HG, SK, DH), BF16),
            pltpu.VMEM((3, B, HG, SK, DH), BF16),
            pltpu.VMEM((3, D, HG * DH), BF16),
            pltpu.VMEM((3, HG * DH, D), BF16),
            pltpu.VMEM((M, D), F32),
            pltpu.VMEM((2, M, D), BF16),
            pltpu.VMEM((sum(FG), M, DH), BF16),
            pltpu.SemaphoreType.DMA((3, 4)),
            pltpu.SemaphoreType.DMA((2, 3)),
            pltpu.SemaphoreType.DMA((XC,)),
            pltpu.SemaphoreType.DMA((FG[0] // 2 + 1,)),
            pltpu.SemaphoreType.DMA((1,)),
            pltpu.SemaphoreType.DMA((1 + len(LCH),)),
        ],
        compiler_params=pltpu.CompilerParams(
            vmem_limit_bytes=100 * 1024 * 1024,
            disable_bounds_checks=True,
            disable_semaphore_checks=True,
        ),
        name="mha2",
    )(A_x.reshape(M, D), A_k_cache, A_v_cache, A_wq, A_wo,
      B_x.reshape(M, D), B_k_cache, B_v_cache, B_wq, B_wo)
    return out.reshape(B, SQ, 2 * D)
```
